```python
import os as _os
_os.environ.setdefault("JAX_PLATFORMS", "cpu")
import jax
import jax.numpy as jnp

def _softmax(x, axis=-1):
    return jax.nn.softmax(x, axis=axis)
def _gelu(x):
    return jax.nn.gelu(x, approximate=True)
def _silu(x):
    return jax.nn.silu(x)
def _sigmoid(x):
    return jax.nn.sigmoid(x)
def _layernorm(x, axis=-1, eps=1e-5):
    m = jnp.mean(x, axis=axis, keepdims=True)
    v = jnp.var(x, axis=axis, keepdims=True)
    return (x - m) / jnp.sqrt(v + eps)
def _scatter_add(tgt, idx, src, axis=0):
    return tgt.at[idx].add(src)
def _segment_sum(src, seg, n):
    return jax.ops.segment_sum(src, seg, n)
class _Rng:
    def __init__(self, key):
        self._k = key
    def _next(self):
        self._k, sub = jax.random.split(self._k)
        return sub
    def normal(self, shape):
        return jax.random.normal(self._next(), shape, dtype=jnp.bfloat16)
    def randint(self, lo, hi, shape):
        return jax.random.randint(self._next(), shape, lo, hi, dtype=jnp.int32)
    def uniform(self, shape, lo=0.0, hi=1.0):
        return jax.random.uniform(self._next(), shape, jnp.bfloat16, lo, hi)
    def permutation(self, n):
        return jax.random.permutation(self._next(), n)


kernel_name = 'concat_heads__sliding_block__ssm_conv_s4__prompt'

def setup_inputs():
    _rng = _Rng(jax.random.key(int.from_bytes(__import__("os").urandom(4), "little")))
    _w = (lambda a: (lambda t: t.astype(jnp.bfloat16) if jnp.issubdtype(t.dtype, jnp.floating) else t)(jnp.asarray(a)))
    def _A_setup():
        B, S, D = 1, 2048, 512
        return {
            "x": _w((lambda *s: _rng.normal(s) * 0.2)(B, S, D)),
            "wqkv": _w((lambda *s: _rng.normal(s) * 0.2)(D, 3 * D)),
            "wo": _w((lambda *s: _rng.normal(s) * 0.05)(D, D)),
        }
    _A_in = _A_setup()

    def _B_setup():
        B, L, D, N = 1, 2048, 512, 128
        A_re = -jnp.exp((lambda *s: _rng.normal(s) * 0.8)(D, N))
        A_im = jnp.pi * (lambda *s: _rng.normal(s) * 0.8)(D, N)
        B_re = (lambda *s: _rng.normal(s) * 0.8)(D, N)
        B_im = (lambda *s: _rng.normal(s) * 0.8)(D, N)
        C_re = (lambda *s: _rng.normal(s) * 0.8)(D, N)
        C_im = (lambda *s: _rng.normal(s) * 0.8)(D, N)
        log_dt = (lambda *s: _rng.normal(s) * 0.8)(D) * 0.5 - 4.0
        Dskip = (lambda *s: _rng.normal(s) * 0.05)(D)
        return {
            "u": _w((lambda *s: _rng.normal(s) * 0.05)(B, L, D)),
            "A_re": _w(A_re),
            "A_im": _w(A_im),
            "B_re": _w(B_re),
            "B_im": _w(B_im),
            "C_re": _w(C_re),
            "C_im": _w(C_im),
            "log_dt": _w(log_dt),
            "Dskip": _w(Dskip),
        }
    _B_in = _B_setup()

    return {
        "A_x": _A_in["x"],
        "A_wqkv": _A_in["wqkv"],
        "A_wo": _A_in["wo"],
        "B_u": _B_in["u"],
        "B_A_re": _B_in["A_re"],
        "B_A_im": _B_in["A_im"],
        "B_B_re": _B_in["B_re"],
        "B_B_im": _B_in["B_im"],
        "B_C_re": _B_in["C_re"],
        "B_C_im": _B_in["C_im"],
        "B_log_dt": _B_in["log_dt"],
        "B_Dskip": _B_in["Dskip"],
    }

def reference(A_x, A_wqkv, A_wo, B_u, B_A_re, B_A_im, B_B_re, B_B_im, B_C_re, B_C_im, B_log_dt, B_Dskip):
    def _A_ref(x, wqkv, wo):
        B, S, D = x.shape
        H = 32; Dh = D // H; W = 256
        qkv = (lambda x, *d: x.transpose(*d))((x @ wqkv).reshape(B, S, 3, H, Dh), 2, 0, 3, 1, 4)
        q, k, v = qkv[0], qkv[1], qkv[2]
        scores = jnp.einsum("bhqd,bhkd->bhqk", q, k) * (Dh ** -0.5)
        idx = jnp.arange(S)
        mask = (idx[:, None] - idx[None, :] >= 0) & (idx[:, None] - idx[None, :] < W)
        scores = jnp.where(mask[None, None], scores, -1e9)
        p = _softmax(scores, axis=-1)
        o = jnp.einsum("bhqk,bhkd->bhqd", p, v)
        return (lambda x, *d: x.transpose(*d))(o, 0, 2, 1, 3).reshape(B, S, D) @ wo

    def _B_ref(u, A_re, A_im, B_re, B_im, C_re, C_im, log_dt, Dskip):
        Bsz, L, D = u.shape
        dt = jnp.exp(log_dt)[:, None]
        A = A_re + 1j * A_im
        Bc = B_re + 1j * B_im
        Cc = C_re + 1j * C_im
        logdA = dt * A
        dB = dt * Bc
        l = (lambda x, dt: x.astype(dt))(jnp.arange(L), A_re.dtype)
        P = jnp.exp(logdA[:, :, None] * l[None, None, :])
        K = jnp.einsum("dn,dnl,dn->dl", Cc, P, dB).real
        L2 = 2 * L
        Kp = jnp.pad(K, ((0, 0), (0, L)))
        up = (lambda x, *d: x.transpose(*d))(u, 0, 2, 1)
        up = jnp.pad(up, ((0, 0), (0, 0), (0, L)))
        Kf = (lambda x, axes=(-2,-1): jnp.fft.rfft2(x.astype(jnp.float32), axes=axes))(Kp[:, None, :], axes=(-2, -1))
        Uf = (lambda x, axes=(-2,-1): jnp.fft.rfft2(x.astype(jnp.float32), axes=axes))(up[:, :, None, :], axes=(-2, -1))
        Yf = Uf * Kf[None, :, :, :]
        y = (lambda x, s, axes=(-2,-1): jnp.fft.irfft2(x, s=s, axes=axes).astype(jnp.bfloat16))(Yf, (1, L2), axes=(-2, -1))[:, :, 0, :L]
        y = (lambda x, *d: x.transpose(*d))(y, 0, 2, 1) + u * Dskip[None, None, :]
        return y

    a = _A_ref(A_x, A_wqkv, A_wo)
    b = _B_ref(B_u, B_A_re, B_A_im, B_B_re, B_B_im, B_C_re, B_C_im, B_log_dt, B_Dskip)
    return jnp.concatenate([a, b], axis=-1)
```

```python
import numpy as np
import jax
import jax.numpy as jnp
import jax.experimental.pallas as pl
import jax.experimental.pallas.tpu as pltpu

S_LEN = 2048
D = 512
NT = 16
NEG = -1e30
bf = jnp.bfloat16
f32 = jnp.float32
i32 = jnp.int32

A_EXP = list(range(16)) + list(range(16, 32, 2)) + list(range(32, 64, 4))
B_EXP = ([16 * b for b in range(16)] + [258 + 32 * b for b in range(8)]
         + [516 + 64 * b for b in range(8)] + [1032 + 64 * b for b in range(16)])
WIN_OF_BLOCK = [0, 1, 2, 3, 4, 5, 5, 5, 6, 7, 7, 7, 7, 7, 7, 7]


def _bf16_bits(x):
    x = np.ascontiguousarray(np.asarray(x, np.float32))
    u = x.view(np.uint32).astype(np.uint64)
    return ((u + 0x7FFF + ((u >> 16) & 1)) >> 16).astype(np.uint32)


def _pack_rows(x):
    b = _bf16_bits(x)
    return (b[0::2] | (b[1::2] << 16)).astype(np.uint32).view(np.int32)


def _windows():
    ai_of = {e: i for i, e in enumerate(A_EXP)}
    W0 = [(ai, 0) for ai in range(16)]
    W1 = [(ai, 8) for ai in range(16)]
    W2 = [(ai_of[e], 16) for e in range(0, 32, 2)]
    W3 = [(ai_of[e], 24) for e in range(0, 64, 4)]
    W4 = [(ai_of[e], 32) for e in range(0, 64, 8)] + [(ai_of[e], 40) for e in range(0, 64, 8)]

    def cols(W):
        return [A_EXP[ai] + B_EXP[b0 + r] for (ai, b0) in W for r in range(8)]
    c2s = cols(W2); c2s[7] = A_EXP[16] + B_EXP[15]
    c3s = cols(W3); c3s[7] = A_EXP[23] + B_EXP[23]
    c4s = cols(W4); c4s[7] = A_EXP[31] + B_EXP[31]
    return [cols(W0), cols(W1), c2s, cols(W2), c3s, cols(W3), c4s, cols(W4)]


def _make_consts():
    k = np.concatenate([np.arange(0, 128, 2), np.arange(1, 128, 2)]).astype(np.float64) + 0.5
    t = np.arange(128, dtype=np.float64)
    th = 2 * np.pi * k[:, None] * t[None, :] / 256
    F = np.concatenate([np.cos(th), -np.sin(th)], axis=0)
    Finv = np.concatenate([np.cos(th).T, -np.sin(th).T], axis=1) / 128
    wins = _windows()
    M = np.zeros((16, 256, 128))
    for i in range(16):
        lag = (_bf16_bits(np.arange(128 * i, 128 * i + 128)) << 16).view(np.float32).astype(np.int64)
        w = wins[WIN_OF_BLOCK[i]]
        for tt in range(128):
            M[i, :, w.index(int(lag[tt]))] += F[:, tt]
    dft = np.concatenate([_pack_rows(F), _pack_rows(Finv[:, :128]), _pack_rows(Finv[:, 128:])], axis=0)
    mm = np.concatenate([_pack_rows(M[i]) for i in range(16)], axis=0)
    return np.ascontiguousarray(dft), np.ascontiguousarray(mm)


_DFT_CONST, _M_CONST = _make_consts()


def _cmul(a, b):
    return (a[0] * b[0] - a[1] * b[1], a[0] * b[1] + a[1] * b[0])


def _cmul_conj(a, b):
    return (a[0] * b[0] + a[1] * b[1], a[1] * b[0] - a[0] * b[1])


def _csq(a):
    return (a[0] * a[0] - a[1] * a[1], 2.0 * (a[0] * a[1]))


def _pk(x, y):
    return pltpu.pack_elementwise([x, y], packed_dtype=bf)


def _sincos(x):
    kf = (x * 0.6366197723675814 + 12582912.0) - 12582912.0
    r = ((x - kf * 1.5703125) - kf * 4.837512969970703125e-4) - kf * 7.54978995489188216e-8
    ki = kf.astype(i32)
    z = r * r
    s = r + (r * z) * (-1.6666654611e-1 + z * (8.3321608736e-3 + z * -1.9515295891e-4))
    c = (1.0 - 0.5 * z) + (z * z) * (4.166664568298827e-2 + z * (-1.388731625493765e-3 + z * 2.443315711809948e-5))
    swap = (ki & 1) != 0
    sn = jnp.where(swap, c, s)
    cs = jnp.where(swap, s, c)
    sbit = jnp.int32(-2 ** 31)
    sn = pltpu.bitcast(pltpu.bitcast(sn, i32) ^ ((ki << 30) & sbit), f32)
    cs = pltpu.bitcast(pltpu.bitcast(cs, i32) ^ (((ki + 1) << 30) & sbit), f32)
    return sn, cs


SR = 33
GCH = 32
NG = D // GCH


def _kernel(x_hbm, wqkv_hbm, wo_hbm, u_hbm, are_hbm, aim_hbm, bre_hbm, bim_hbm, cre_hbm, cim_hbm,
            ldt_hbm, dsk_hbm, dft_hbm, mm_hbm,
            out_hbm,
            XB, UB, WB, WOB, PAR, LDT, DSK, DFT, MM,
            WQT, WKP, WVT, WOP, XP,
            QT, KS, VT, OT, SA, SB, BIAS,
            ZC, TAB, XG, GW, KH, UH, TH, OUT,
            sems, osems):
    par_src = [are_hbm, aim_hbm, bre_hbm, bim_hbm, cre_hbm, cim_hbm]
    cp_par = [pltpu.make_async_copy(par_src[i], PAR.at[i], sems.at[i]) for i in range(6)]
    cp_ldt = pltpu.make_async_copy(ldt_hbm, LDT, sems.at[6])
    cp_dsk = pltpu.make_async_copy(dsk_hbm, DSK, sems.at[7])
    cp_w = pltpu.make_async_copy(wqkv_hbm, WB, sems.at[8])
    cp_x = [pltpu.make_async_copy(x_hbm.at[pl.ds(512 * i, 512)], XB.at[pl.ds(512 * i, 512)], sems.at[9 + i])
            for i in range(4)]
    cp_u = pltpu.make_async_copy(u_hbm, UB, sems.at[13])
    cp_wo = pltpu.make_async_copy(wo_hbm, WOB, sems.at[14])
    cp_dft = pltpu.make_async_copy(dft_hbm, DFT, sems.at[15])
    cp_mm = pltpu.make_async_copy(mm_hbm, MM, sems.at[16])
    cp_ldt.start()
    for c in cp_par:
        c.start()
    cp_w.start()
    cp_x[0].start()

    def bias_init():
        kk = jax.lax.broadcasted_iota(i32, (128, 128), 0)
        qq = jax.lax.broadcasted_iota(i32, (128, 128), 1)
        BIAS[0] = jnp.where(kk > qq, 0.0, NEG).astype(f32)
        BIAS[1] = jnp.where(kk <= qq, 0.0, NEG).astype(f32)

    def t0(c):
        dtr = LDT[...].astype(f32).reshape(1, D)
        dtr = jnp.exp(dtr[:, 128 * c:128 * (c + 1)]).astype(bf).astype(f32)
        dtc = jnp.broadcast_to(dtr, (128, 128)).T
        for b in range(8):
            rows = pl.ds(128 * c + 16 * b, 16)
            dt = dtc[16 * b:16 * (b + 1)]
            are = PAR[0, rows, :].astype(f32); aim = PAR[1, rows, :].astype(f32)
            bre = PAR[2, rows, :].astype(f32) * dt; bim = PAR[3, rows, :].astype(f32) * dt
            cre = PAR[4, rows, :].astype(f32); cim = PAR[5, rows, :].astype(f32)
            mag = jnp.exp(dt * are)
            sn, cs = _sincos(dt * aim)
            ZC[0, rows, :] = mag * cs
            ZC[1, rows, :] = mag * sn
            ZC[2, rows, :] = cre * bre - cim * bim
            ZC[3, rows, :] = -(cre * bim + cim * bre)

    def t1_tables(g):
        buf = g % 2
        for blk in range(GCH // 16):
            rows = pl.ds(g * GCH + 16 * blk, 16)
            z = (ZC[0, rows, :], ZC[1, rows, :])
            cur = (ZC[2, rows, :], ZC[3, rows, :])

            def store(base, q, v0, v1, blk=blk):
                TAB[buf, 0, pl.ds((base + q) * SR + 16 * blk, 16), :] = _pk(v0[0], v1[0])
                TAB[buf, 1, pl.ds((base + q) * SR + 16 * blk, 16), :] = _pk(v0[1], v1[1])
            z2 = _csq(z); z4 = _csq(z2); z8 = _csq(z4); z16 = _csq(z8); z32 = _csq(z16); z64 = _csq(z32)
            vals = [cur]
            for _ in range(16):
                cur = _cmul_conj(cur, z); vals.append(cur)
            for _ in range(8):
                cur = _cmul_conj(cur, z2); vals.append(cur)
            for _ in range(7):
                cur = _cmul_conj(cur, z4); vals.append(cur)
            for q in range(16):
                store(0, q, vals[2 * q], vals[2 * q + 1])
            vb = [(jnp.ones_like(z[0]), jnp.zeros_like(z[0])), z16, z32]
            cur = z32
            for b in range(3, 16):
                cur = z64 if b == 4 else _cmul(cur, z16)
                vb.append(cur)
            cur = _cmul(_cmul(cur, z16), z2)
            z258 = cur
            vb.append(cur)
            for _ in range(7):
                cur = _cmul(cur, z32); vb.append(cur)
            cur = _csq(z258); z516 = cur
            vb.append(cur)
            for _ in range(7):
                cur = _cmul(cur, z64); vb.append(cur)
            cur = _csq(z516)
            vb.append(cur)
            for _ in range(15):
                cur = _cmul(cur, z64); vb.append(cur)
            for q in range(24):
                store(16, q, vb[2 * q], vb[2 * q + 1])

    def t1_vand(g, d0, d1):
        buf = g % 2
        for d in range(d0, d1):
            def ld(ri, base, n):
                return jnp.concatenate(
                    [pltpu.bitcast(TAB[buf, ri, pl.ds((base + 8 * j) * SR + d, 8, stride=SR), :], bf)
                     for j in range(n)], axis=0)
            a = jnp.concatenate([ld(0, 0, 2), ld(1, 0, 2)], axis=1)
            b = jnp.concatenate([ld(0, 16, 3), ld(1, 16, 3)], axis=1)
            o = jax.lax.dot_general(a, b, (((1,), (1,)), ((), ())), preferred_element_type=f32)
            XG[pl.ds((g * GCH + d) * SR, 32), pl.ds(0, 48)] = o

    def t2(c):
        sub7 = jax.lax.broadcasted_iota(i32, (8, 128), 0) == 7
        pend = {}

        def put(w, grp, val):
            key = (w, grp // 2)
            if key in pend:
                other = pend.pop(key)
                lo, hi = (other, val) if grp % 2 else (val, other)
                GW[c, w, pl.ds(8 * (grp // 2), 8), :] = pltpu.bitcast(
                    jnp.concatenate([lo, hi], axis=0).astype(bf), i32)
                return lo, hi
            pend[key] = val
            return None
        keep = {}
        for ai in range(32):
            e = A_EXP[ai]
            tt = XG[pl.ds(128 * c * SR + ai, 128, stride=SR), pl.ds(0, 48)].T
            if ai < 16:
                put(0, ai, tt[0:8]); put(1, ai, tt[8:16])
            if e % 2 == 0 and e < 32:
                r = put(3, e // 2, tt[16:24])
                if r is not None and e == 2:
                    keep['w2'] = r
            if e % 4 == 0:
                r = put(5, e // 4, tt[24:32])
                if r is not None and e == 4:
                    keep['w3'] = r
            if e % 8 == 0:
                r = put(7, e // 8, tt[32:40])
                if r is not None and e == 8:
                    keep['w4'] = r
                put(7, 8 + e // 8, tt[40:48])
            if ai == 16:
                keep['e2'] = tt[8:16]
            if ai == 23:
                keep['e3'] = tt[16:24]
            if ai == 31:
                keep['e4'] = tt[24:32]
        assert not pend
        for (ws, wn, kw, ke) in ((2, 3, 'w2', 'e2'), (4, 5, 'w3', 'e3'), (6, 7, 'w4', 'e4')):
            lo, hi = keep[kw]
            lo = jnp.where(sub7, keep[ke], lo)
            GW[c, ws, pl.ds(0, 8), :] = pltpu.bitcast(jnp.concatenate([lo, hi], axis=0).astype(bf), i32)
            GW[c, ws, pl.ds(8, 56), :] = GW[c, wn, pl.ds(8, 56), :]

    def t3(c, i):
        m = pltpu.bitcast(MM[pl.ds(128 * i, 128), :], bf)
        w = pltpu.bitcast(GW[c, WIN_OF_BLOCK[i]], bf)
        KH[c, i] = jnp.dot(m, w, preferred_element_type=f32)

    def t4(c, m):
        fm = pltpu.bitcast(DFT[pl.ds(0, 128), :], bf)
        w = UB[pl.ds(128 * m, 128), pl.ds(128 * c, 128)]
        UH[c, m] = jnp.dot(fm, w, preferred_element_type=f32)

    def t5(c, hp):
        re = pl.ds(16 * hp, 16); im = pl.ds(128 + 16 * hp, 16)
        sg = hp < 4
        prev = None
        for j in range(16):
            ar = ai = None
            for i in range(j + 1):
                kr = KH[c, i, re, :]; ki = KH[c, i, im, :]
                ur = UH[c, j - i, re, :]; ui = UH[c, j - i, im, :]
                pr = kr * ur - ki * ui
                pi = kr * ui + ki * ur
                ar = pr if ar is None else ar + pr
                ai = pi if ai is None else ai + pi
            if prev is None:
                tr, ti = ar, ai
            elif sg:
                tr, ti = ar - prev[1], ai + prev[0]
            else:
                tr, ti = ar + prev[1], ai - prev[0]
            prev = (ar, ai)
            TH[c, j, pl.ds(8 * hp, 8), :] = pltpu.bitcast(tr.astype(bf), i32)
            TH[c, j, pl.ds(64 + 8 * hp, 8), :] = pltpu.bitcast(ti.astype(bf), i32)

    def t6(c, j):
        fi = jnp.concatenate([pltpu.bitcast(DFT[pl.ds(128, 64), :], bf),
                              pltpu.bitcast(DFT[pl.ds(192, 64), :], bf)], axis=1)
        w = pltpu.bitcast(TH[c, j], bf)
        y = jnp.dot(fi, w, preferred_element_type=f32)
        uu = UB[pl.ds(128 * j, 128), pl.ds(128 * c, 128)].astype(f32)
        dsk = DSK[...].astype(f32).reshape(1, D)[:, 128 * c:128 * (c + 1)]
        OUT[pl.ds(128 * j, 128), pl.ds(512 + 128 * c, 128)] = (y + uu * dsk).astype(bf)

    def relayout_qkv():
        for (dst, off) in ((WQT, 0), (WVT, 1024)):
            for a in range(4):
                for b in range(4):
                    t = WB[pl.ds(128 * b, 128), pl.ds(off + 128 * a, 128)].T
                    dst[pl.ds(64 * a, 64), pl.ds(128 * b, 128)] = pltpu.bitcast(t, i32)
        for b in range(4):
            WKP[:, pl.ds(128 * b, 128)] = pltpu.bitcast(WB[:, pl.ds(512 + 128 * b, 128)], i32)

    def relayout_wo():
        for b in range(4):
            WOP[:, pl.ds(128 * b, 128)] = pltpu.bitcast(WOB[:, pl.ds(128 * b, 128)], i32)

    def proj_x(j):
        for b in range(4):
            XP[j % 2, :, pl.ds(128 * b, 128)] = pltpu.bitcast(XB[pl.ds(128 * j, 128), pl.ds(128 * b, 128)], i32)

    def proj_k(j, g):
        xb = pltpu.bitcast(XP[j % 2], bf)
        w = pltpu.bitcast(WKP[:, pl.ds(128 * g, 128)], bf)
        k = jnp.dot(xb, w, preferred_element_type=f32)
        KS[g, pl.ds(64 * j, 64), :] = pltpu.bitcast(k.astype(bf), i32)

    qscale = float(0.25 * np.log2(np.e))

    def proj_t(j, g, which):
        xb = pltpu.bitcast(XP[j % 2], bf)
        wt = pltpu.bitcast((WQT if which == 'q' else WVT)[pl.ds(64 * g, 64), :], bf)
        r = jax.lax.dot_general(wt, xb, (((1,), (1,)), ((), ())), preferred_element_type=f32)
        if which == 'q':
            QT[j, pl.ds(64 * g, 64), :] = pltpu.bitcast((r * qscale).astype(bf), i32)
        else:
            VT[j, pl.ds(64 * g, 64), :] = pltpu.bitcast(r.astype(bf), i32)

    zeros16 = jnp.zeros((16, 128), bf)

    def prod_unit(qi, h, kt, S, slot, macc):
        g, hh = h // 8, h % 8
        kb = qi - 2 + kt
        kk = pltpu.bitcast(KS[g, pl.ds(64 * kb, 64), :], bf)
        qh = pltpu.bitcast(QT[qi, pl.ds(8 * h, 8), :], bf)
        w = jnp.concatenate([zeros16] * hh + [qh] + [zeros16] * (7 - hh), axis=0)
        s = jnp.dot(kk, w, preferred_element_type=f32)
        if kt != 1:
            s = s + BIAS[kt // 2]
        S[slot] = s
        pm = jnp.max(s.reshape(16, 8, 128), axis=0)
        return pm if macc is None else jnp.maximum(macc, pm)

    def cons_unit(qi, h, kt, S, slot, m, lacc, oacc):
        kb = qi - 2 + kt
        p = jnp.exp2(S[slot] - m)
        ps = jnp.sum(p.reshape(16, 8, 128), axis=0)
        lacc = ps if lacc is None else lacc + ps
        v = pltpu.bitcast(VT[kb, pl.ds(8 * h, 8), :], bf)
        o = jnp.dot(v, p.astype(bf), preferred_element_type=f32)
        oacc = o if oacc is None else oacc + o
        return lacc, oacc

    def kts(qi):
        return [kt for kt in range(3) if qi - 2 + kt >= 0]

    def group(pitem, Sp, citem, Sc, ms):
        new_ms = []
        for t in range(4):
            macc = lacc = oacc = None
            pk_ = kts(pitem[0]) if pitem is not None else []
            ck_ = kts(citem[0]) if citem is not None else []
            for n in range(max(len(pk_), len(ck_))):
                if n < len(pk_):
                    macc = prod_unit(pitem[0], 4 * pitem[1] + t, pk_[n], Sp, 3 * t + pk_[n], macc)
                if n < len(ck_):
                    lacc, oacc = cons_unit(citem[0], 4 * citem[1] + t, ck_[n], Sc, 3 * t + ck_[n], ms[t], lacc, oacc)
            if pitem is not None:
                new_ms.append(jnp.max(macc, axis=0, keepdims=True))
            if citem is not None:
                l = jnp.sum(lacc, axis=0, keepdims=True)
                o = oacc * pl.reciprocal(l, approx=True)
                h = 4 * citem[1] + t
                OT[citem[0], pl.ds(8 * h, 8), :] = pltpu.bitcast(o.astype(bf), i32)
        return new_ms

    def out_proj(i):
        o = jnp.concatenate([pltpu.bitcast(OT[i, pl.ds(64 * g, 64), :], bf).T for g in range(4)], axis=1)
        r = jnp.dot(o, pltpu.bitcast(WOP[...], bf), preferred_element_type=f32)
        OUT[pl.ds(128 * i, 128), pl.ds(0, 512)] = r.astype(bf)

    out_copies = []

    def out_dma(r0, nr, c0, nc):
        cp = pltpu.make_async_copy(OUT.at[pl.ds(r0, nr), pl.ds(c0, nc)],
                                   out_hbm.at[pl.ds(r0, nr), pl.ds(c0, nc)], osems.at[len(out_copies)])
        cp.start()
        out_copies.append(cp)

    bias_init()
    cp_ldt.wait()
    for c in cp_par:
        c.wait()
    cp_x[1].start()
    cp_dft.start()
    cp_u.start()
    for c in range(4):
        t0(c)
    t1_tables(0)
    cp_w.wait()
    relayout_qkv()
    cp_x[2].start()
    cp_x[3].start()
    cp_mm.start()
    cp_wo.start()
    cp_dsk.start()
    for j in range(16):
        if j % 4 == 0:
            cp_x[j // 4].wait()
        proj_x(j)
        if j + 1 < NG:
            t1_tables(j + 1)
        for g in range(4):
            proj_k(j, g)
            proj_t(j, g, 'q')
            proj_t(j, g, 'v')
            t1_vand(j, 8 * g, 8 * g + 8)
        if j % 4 == 0 and j > 0:
            t2(j // 4 - 1)
        if j == 4:
            cp_dft.wait()
            cp_u.wait()
        if j == 8:
            cp_mm.wait()
        if j >= 4:
            lo = (j - 4) * 64 // 12; hi = (j - 3) * 64 // 12
            for n in range(lo, hi):
                t4(n // 16, n % 16)
        if j >= 8:
            for n in range(4 * (j - 8), 4 * (j - 8) + 4):
                t3(n // 16, n % 16)
        if j >= 12:
            t5(0, 2 * (j - 12)); t5(0, 2 * (j - 12) + 1)
    cp_wo.wait()
    cp_dsk.wait()
    relayout_wo()
    items = [(qi, hg) for qi in range(16) for hg in range(8)]
    ms = group(items[0], SA, None, None, None)
    bufs = [SA, SB]
    for n, it in enumerate(items):
        nxt = items[n + 1] if n + 1 < len(items) else None
        ms = group(nxt, bufs[(n + 1) % 2], it, bufs[n % 2], ms)
        qi, hg = it
        s = qi
        if hg == 0 and s == 0:
            t2(3)
        if hg == 1 and s < 8:
            for m in range(32 + 4 * s, 32 + 4 * s + 4):
                t3(m // 16, m % 16)
        if hg in (2, 5) and s < 12:
            t5(1 + s // 4, 2 * (s % 4) + (hg == 5))
        if hg == 3:
            c, q4 = s // 4, s % 4
            for j in range(4 * q4, 4 * q4 + 4):
                t6(c, j)
        if hg == 4:
            c, q4 = s // 4, s % 4
            out_dma(512 * q4, 512, 512 + 128 * c, 128)
        if hg == 0 and s > 0:
            out_proj(s - 1)
        if hg == 1 and s > 0:
            out_dma(128 * (s - 1), 128, 0, 512)
    out_proj(15)
    out_dma(128 * 15, 128, 0, 512)
    for cp in out_copies:
        cp.wait()


@jax.jit
def pallas_concat_heads__sliding_block__ssm_conv_s4__prompt_kernel(A_x, A_wqkv, A_wo, B_u, B_A_re, B_A_im, B_B_re, B_B_im, B_C_re, B_C_im, B_log_dt, B_Dskip):
    any_spec = pl.BlockSpec(memory_space=pl.ANY)
    scratch = [
        pltpu.VMEM((S_LEN, D), bf), pltpu.VMEM((S_LEN, D), bf), pltpu.VMEM((D, 3 * D), bf), pltpu.VMEM((D, D), bf),
        pltpu.VMEM((6, D, 128), bf), pltpu.VMEM((D,), bf), pltpu.VMEM((D,), bf),
        pltpu.VMEM((256, 128), i32), pltpu.VMEM((2048, 128), i32),
        pltpu.VMEM((256, D), i32), pltpu.VMEM((256, D), i32), pltpu.VMEM((256, D), i32), pltpu.VMEM((256, D), i32),
        pltpu.VMEM((2, 64, D), i32),
        pltpu.VMEM((NT, 256, 128), i32), pltpu.VMEM((4, 1024, 128), i32), pltpu.VMEM((NT, 256, 128), i32),
        pltpu.VMEM((NT, 256, 128), i32), pltpu.VMEM((12, 128, 128), f32), pltpu.VMEM((12, 128, 128), f32),
        pltpu.VMEM((2, 128, 128), f32),
        pltpu.VMEM((4, D, 128), f32), pltpu.VMEM((2, 2, 40 * SR, 128), i32), pltpu.VMEM((D * SR, 128), f32),
        pltpu.VMEM((4, 8, 64, 128), i32), pltpu.VMEM((4, NT, 256, 128), f32), pltpu.VMEM((4, NT, 256, 128), f32),
        pltpu.VMEM((4, NT, 128, 128), i32), pltpu.VMEM((S_LEN, 2 * D), bf),
        pltpu.SemaphoreType.DMA((17,)), pltpu.SemaphoreType.DMA((32,)),
    ]
    out = pl.pallas_call(
        _kernel,
        out_shape=jax.ShapeDtypeStruct((S_LEN, 2 * D), bf),
        in_specs=[any_spec] * 14,
        out_specs=any_spec,
        scratch_shapes=scratch,
        compiler_params=pltpu.CompilerParams(vmem_limit_bytes=110 * 1024 * 1024),
        name="fused_swa_s4",
    )(A_x.reshape(S_LEN, D), A_wqkv, A_wo, B_u.reshape(S_LEN, D), B_A_re, B_A_im, B_B_re, B_B_im, B_C_re, B_C_im,
      B_log_dt, B_Dskip, _DFT_CONST, _M_CONST)
    return out.reshape(1, S_LEN, 2 * D)
```

```python
import numpy as np
import jax
import jax.numpy as jnp
import jax.experimental.pallas as pl
import jax.experimental.pallas.tpu as pltpu

S_LEN = 2048
D = 512
NT = 16
NEG = -1e30
bf = jnp.bfloat16
f32 = jnp.float32
i32 = jnp.int32

A_EXP = list(range(16)) + list(range(16, 32, 2)) + list(range(32, 64, 4))
B_EXP = ([16 * b for b in range(16)] + [258 + 32 * b for b in range(8)]
         + [516 + 64 * b for b in range(8)] + [1032 + 64 * b for b in range(16)])
WIN_OF_BLOCK = [0, 1, 2, 3, 4, 5, 5, 5, 6, 7, 7, 7, 7, 7, 7, 7]


def _bf16_bits(x):
    x = np.ascontiguousarray(np.asarray(x, np.float32))
    u = x.view(np.uint32).astype(np.uint64)
    return ((u + 0x7FFF + ((u >> 16) & 1)) >> 16).astype(np.uint32)


def _pack_rows(x):
    b = _bf16_bits(x)
    return (b[0::2] | (b[1::2] << 16)).astype(np.uint32).view(np.int32)


def _windows():
    ai_of = {e: i for i, e in enumerate(A_EXP)}
    W0 = [(ai, 0) for ai in range(16)]
    W1 = [(ai, 8) for ai in range(16)]
    W2 = [(ai_of[e], 16) for e in range(0, 32, 2)]
    W3 = [(ai_of[e], 24) for e in range(0, 64, 4)]
    W4 = [(ai_of[e], 32) for e in range(0, 64, 8)] + [(ai_of[e], 40) for e in range(0, 64, 8)]

    def cols(W):
        return [A_EXP[ai] + B_EXP[b0 + r] for (ai, b0) in W for r in range(8)]
    c2s = cols(W2); c2s[7] = A_EXP[16] + B_EXP[15]
    c3s = cols(W3); c3s[7] = A_EXP[23] + B_EXP[23]
    c4s = cols(W4); c4s[7] = A_EXP[31] + B_EXP[31]
    return [cols(W0), cols(W1), c2s, cols(W2), c3s, cols(W3), c4s, cols(W4)]


def _make_consts():
    k = np.concatenate([np.arange(0, 128, 2), np.arange(1, 128, 2)]).astype(np.float64) + 0.5
    t = np.arange(128, dtype=np.float64)
    th = 2 * np.pi * k[:, None] * t[None, :] / 256
    F = np.concatenate([np.cos(th), -np.sin(th)], axis=0)
    Finv = np.concatenate([np.cos(th).T, -np.sin(th).T], axis=1) / 128
    wins = _windows()
    M = np.zeros((16, 256, 128))
    for i in range(16):
        lag = (_bf16_bits(np.arange(128 * i, 128 * i + 128)) << 16).view(np.float32).astype(np.int64)
        w = wins[WIN_OF_BLOCK[i]]
        for tt in range(128):
            M[i, :, w.index(int(lag[tt]))] += F[:, tt]
    dft = np.concatenate([_pack_rows(F), _pack_rows(Finv[:, :128]), _pack_rows(Finv[:, 128:])], axis=0)
    mm = np.concatenate([_pack_rows(M[i]) for i in range(16)], axis=0)
    return np.ascontiguousarray(dft), np.ascontiguousarray(mm)


_DFT_CONST, _M_CONST = _make_consts()
_ZERO = np.zeros((8,), np.int32)


def _cmul(a, b):
    return (a[0] * b[0] - a[1] * b[1], a[0] * b[1] + a[1] * b[0])


def _cmul_conj(a, b):
    return (a[0] * b[0] + a[1] * b[1], a[1] * b[0] - a[0] * b[1])


def _csq(a):
    return (a[0] * a[0] - a[1] * a[1], 2.0 * (a[0] * a[1]))


def _pk(x, y):
    return pltpu.pack_elementwise([x, y], packed_dtype=bf)


def _sincos(x):
    kf = (x * 0.6366197723675814 + 12582912.0) - 12582912.0
    r = ((x - kf * 1.5703125) - kf * 4.837512969970703125e-4) - kf * 7.54978995489188216e-8
    ki = kf.astype(i32)
    z = r * r
    s = r + (r * z) * (-1.6666654611e-1 + z * (8.3321608736e-3 + z * -1.9515295891e-4))
    c = (1.0 - 0.5 * z) + (z * z) * (4.166664568298827e-2 + z * (-1.388731625493765e-3 + z * 2.443315711809948e-5))
    swap = (ki & 1) != 0
    sn = jnp.where(swap, c, s)
    cs = jnp.where(swap, s, c)
    sbit = jnp.int32(-2 ** 31)
    sn = pltpu.bitcast(pltpu.bitcast(sn, i32) ^ ((ki << 30) & sbit), f32)
    cs = pltpu.bitcast(pltpu.bitcast(cs, i32) ^ (((ki + 1) << 30) & sbit), f32)
    return sn, cs


SR = 33
GCH = 32
NG = D // GCH
NTB = 6
TB = 16
THROTTLE = True
ZOFF = D * SR
UNROLL = 7
SPLIT = 0
RR = False
FLAGS = {}
FILL = 64
BAR = 0
B_RATE = 6


def _ds(start, n):
    return pl.ds(start if isinstance(start, int) else pl.multiple_of(start, n), n)


def _v(ref):
    return ref.bitcast(i32)


def _ld(view, *idx):
    return pltpu.bitcast(view[idx], bf)


SCHED = [
    dict(vs=(2, 3), tabs=(4, 5, 6)),
    dict(vs=(4, 5, 6), tabs=(7, 8, 9)),
    dict(vs=(7, 8, 9), tabs=(10, 11, 12)),
    dict(wait=('u',), vs=(10, 11, 12), tabs=(13, 14, 15), t2s=(0,), d34=(0,)),
    dict(vs=(13, 14, 15), d34=(1,), macs=((0, 3),)),
    dict(p=1, nok=True, t2s=(2,), d34=(2,), macs=((0, 3), (1, 3))),
    dict(p=2, nok=True, d34=(3,), macs=((0, 3), (1, 3))),
    dict(p=3, nok=True, macs=((0, 2), (1, 2))),
    dict(wait=('x2', 'wo'), p=4, macs=((0, 2), (1, 2), (2, 1))),
    dict(p=5, macs=((0, 2), (1, 2), (2, 1))),
    dict(p=6, macs=((0, 1), (1, 2), (2, 2))),
    dict(p=7, macs=((1, 2), (2, 2)), t6s=((0, 0, 8),)),
    dict(wait=('x3',), p=8, macs=((2, 2), (3, 2)), t6s=((0, 8, 16),)),
    dict(p=9, macs=((2, 2), (3, 2)), t6s=((1, 0, 8),)),
    dict(p=10, macs=((2, 2), (3, 2)), t6s=((1, 8, 16),)),
    dict(p=11, macs=((2, 2), (3, 2))),
    dict(p=12, macs=((2, 2), (3, 2))),
    dict(p=13, macs=((3, 2),), t6s=((2, 0, 8),)),
    dict(p=14, macs=((3, 2),), t6s=((2, 8, 16),)),
    dict(p=15, macs=((3, 2),), wot=True),
]
Q0_ROWS = 2
GS = 4
PAIR = True
FULL = False
CONS_FIRST = False
KT_ORDER = [0, 1, 2]


def _kernel(zero_ref, x_hbm, wqkv_hbm, wo_hbm, u_hbm, are_hbm, aim_hbm, bre_hbm, bim_hbm, cre_hbm, cim_hbm,
            ldt_hbm, dsk_hbm, dft_hbm, mm_hbm,
            out_hbm,
            XB, UB, WB, WOB, PAR, LDT, DSK, DFT, MM,
            WQT, WVT, WOT,
            QT, KS, KR, VT, OT, SA, SB, BIAS,
            TAB, XG, XT, KH, UH, DSKB, OUT,
            sems, osems):
    z0 = zero_ref[0]
    XBv, UBv, WBv, WOBv = _v(XB), _v(UB), _v(WB), _v(WOB)
    WQTv, WVTv, WOTv = _v(WQT), _v(WVT), _v(WOT)
    QTv, KSv, KRv, VTv, OTv = _v(QT), _v(KS), _v(KR), _v(VT), _v(OT)
    nsem = [0]

    def mk(src, dst):
        cp = pltpu.make_async_copy(src, dst, sems.at[nsem[0]])
        nsem[0] += 1
        return cp
    par_src = [are_hbm, aim_hbm, bre_hbm, bim_hbm, cre_hbm, cim_hbm]
    cp_par = [mk(par_src[i], PAR.at[i]) for i in range(6)]
    cp_ldt = mk(ldt_hbm, LDT)
    cp_dsk = mk(dsk_hbm, DSK)
    cp_w = [mk(wqkv_hbm.at[:, pl.ds(128 * t, 128)], WB.at[t]) for t in range(12)]
    x_chunks = [(0, 128), (128, 384), (512, 512), (1024, 1024)]
    cp_x = [[mk(x_hbm.at[pl.ds(r0, nr), pl.ds(128 * b, 128)], XB.at[b, pl.ds(r0, nr)])
             for b in range(4)] for (r0, nr) in x_chunks]
    cp_u = [mk(u_hbm.at[:, pl.ds(128 * b, 128)], UB.at[b]) for b in range(4)]
    cp_wo = [mk(wo_hbm.at[:, pl.ds(128 * b, 128)], WOB.at[b]) for b in range(4)]
    cp_dft = mk(dft_hbm, DFT)
    cp_mm = mk(mm_hbm, MM)

    def start(l):
        for c in l:
            c.start()

    def wait(l):
        for c in l:
            c.wait()

    def bias_init():
        kk = jax.lax.broadcasted_iota(i32, (128, 128), 0)
        qq = jax.lax.broadcasted_iota(i32, (128, 128), 1)
        BIAS[0] = jnp.where(kk > qq, 0.0, NEG).astype(f32)
        BIAS[1] = jnp.where(kk <= qq, 0.0, NEG).astype(f32)
        BIAS[2] = jnp.where(kk < 64, jnp.where(kk <= qq, 0.0, NEG), jnp.where(kk > qq, 0.0, NEG)).astype(f32)
        BIAS[3] = jnp.where(qq < 64, jnp.where(kk > qq, 0.0, NEG), jnp.where(kk + 64 <= qq, 0.0, NEG)).astype(f32)

    def t0(c):
        dtr = LDT[...].astype(f32).reshape(1, D)
        dtr = jnp.exp(dtr[:, 128 * c:128 * (c + 1)]).astype(bf).astype(f32)
        dtc = jnp.broadcast_to(dtr, (128, 128)).T
        for b in range(8):
            rows = pl.ds(128 * c + 16 * b, 16)
            dt = dtc[16 * b:16 * (b + 1)]
            are = PAR[0, rows, :].astype(f32); aim = PAR[1, rows, :].astype(f32)
            bre = PAR[2, rows, :].astype(f32) * dt; bim = PAR[3, rows, :].astype(f32) * dt
            cre = PAR[4, rows, :].astype(f32); cim = PAR[5, rows, :].astype(f32)
            mag = jnp.exp(dt * are)
            sn, cs = _sincos(dt * aim)
            r0 = ZOFF + 128 * c + 16 * b
            XG[pl.ds(r0, 16), :] = mag * cs
            XG[pl.ds(r0 + D, 16), :] = mag * sn
            XG[pl.ds(r0 + 2 * D, 16), :] = cre * bre - cim * bim
            XG[pl.ds(r0 + 3 * D, 16), :] = -(cre * bim + cim * bre)

    def t1_tables(g):
        buf = g % NTB
        for blk in range(GCH // TB):
            r0 = ZOFF + (256 * (g // 8) + 128 * blk + 16 * (g % 8) if PAIR else g * GCH + TB * blk)

            def zc(k, r0=r0):
                if THROTTLE:
                    return XG[pl.ds(pl.multiple_of(8 * z0 + (r0 + k * D), 8), TB), :]
                return XG[pl.ds(r0 + k * D, TB), :]
            z = (zc(0), zc(1))
            cur = (zc(2), zc(3))
            pend = []

            def emit(base, idx, v, blk=blk, pend=pend):
                if idx % 2 == 0:
                    pend.append(v)
                else:
                    v0 = pend.pop()
                    q = base + idx // 2
                    TAB[buf, 0, pl.ds(q * SR + TB * blk, TB), :] = _pk(v0[0], v[0])
                    TAB[buf, 1, pl.ds(q * SR + TB * blk, TB), :] = _pk(v0[1], v[1])
            z2 = _csq(z); z4 = _csq(z2)
            n = 0
            emit(0, n, cur); n += 1
            for (mult, cnt) in ((z, 16), (z2, 8), (z4, 7)):
                for _ in range(cnt):
                    cur = _cmul_conj(cur, mult)
                    emit(0, n, cur); n += 1
            z8 = _csq(z4); z16 = _csq(z8); z32 = _csq(z16)
            n = 0
            emit(16, n, (jnp.ones_like(z[0]), jnp.zeros_like(z[0]))); n += 1
            emit(16, n, z16); n += 1
            emit(16, n, z32); n += 1
            cur = z32
            for b in range(3, 16):
                cur = _cmul(cur, z16)
                if b == 4:
                    z64 = cur
                emit(16, n, cur); n += 1
            cur = _cmul(_cmul(cur, z16), z2)
            z258 = cur
            emit(16, n, cur); n += 1
            for _ in range(7):
                cur = _cmul(cur, z32)
                emit(16, n, cur); n += 1
            cur = _csq(z258); z516 = cur
            emit(16, n, cur); n += 1
            for _ in range(7):
                cur = _cmul(cur, z64)
                emit(16, n, cur); n += 1
            cur = _csq(z516)
            emit(16, n, cur); n += 1
            for _ in range(15):
                cur = _cmul(cur, z64)
                emit(16, n, cur); n += 1

    def t1_vand(g, d0, d1):
        buf = g % NTB

        def ld(ri, base, n, d):
            return jnp.concatenate(
                [pltpu.bitcast(TAB[buf, ri, pl.ds((base + 8 * j) * SR + d, 8, stride=SR), :], bf)
                 for j in range(n)], axis=0)

        def ab(d):
            return (jnp.concatenate([ld(0, 0, 2, d), ld(1, 0, 2, d)], axis=1),
                    jnp.concatenate([ld(0, 16, 3, d), ld(1, 16, 3, d)], axis=1))
        nt = (((1,), (1,)), ((), ()))
        if PAIR:
            z16 = jnp.zeros((16, 256), bf)
            lo = jax.lax.broadcasted_iota(i32, (32, 128), 1) < 64
            for d in range(d0 // 2, d1 // 2):
                a0, b0 = ab(d)
                a1, b1 = ab(16 + d)
                o = jax.lax.dot_general(jnp.concatenate([a0, a1], axis=0),
                                        jnp.concatenate([b0, z16, b1, z16], axis=0), nt,
                                        preferred_element_type=f32)
                XG[pl.ds((128 * (g // 8) + 16 * (g % 8) + d) * SR, 32), :] = jnp.where(lo, o[0:32], o[32:64])
            return
        for d in range(d0, d1):
            a, b = ab(d)
            XG[pl.ds((g * GCH + d) * SR, 32), pl.ds(0, 48)] = jax.lax.dot_general(a, b, nt, preferred_element_type=f32)

    def t2(c, ai):
        if PAIR:
            if c % 2 == 1:
                return
            tt = XG[pl.ds(128 * (c // 2) * SR + ai, 128, stride=SR), :].T
            XT[c, ai] = tt[0:48]
            XT[c + 1, ai] = tt[64:112]
        else:
            XT[c, ai] = XG[pl.ds(128 * c * SR + ai, 128, stride=SR), pl.ds(0, 48)].T

    ai_of = {e: i for i, e in enumerate(A_EXP)}
    wgroups = [[(ai, 0) for ai in range(16)], [(ai, 8) for ai in range(16)],
               [(ai_of[e], 16) for e in range(0, 32, 2)], [(ai_of[e], 24) for e in range(0, 64, 4)],
               [(ai_of[e], 32) for e in range(0, 64, 8)] + [(ai_of[e], 40) for e in range(0, 64, 8)]]
    wins = [(wgroups[0], None), (wgroups[1], None), (wgroups[2], (16, 8)), (wgroups[2], None),
            (wgroups[3], (23, 16)), (wgroups[3], None), (wgroups[4], (31, 24)), (wgroups[4], None)]

    def t3(c, i):
        grp, edge = wins[WIN_OF_BLOCK[i]]
        parts = [XT[c, ai, pl.ds(b0, 8), :] for (ai, b0) in grp]
        if edge is not None:
            sub7 = jax.lax.broadcasted_iota(i32, (8, 128), 0) == 7
            parts[0] = jnp.where(sub7, XT[c, edge[0], pl.ds(edge[1], 8), :], parts[0])
        w = jnp.concatenate(parts, axis=0).astype(bf)
        m = pltpu.bitcast(MM[pl.ds(128 * i, 128), :], bf)
        KH[24 * c + i] = jnp.dot(m, w, preferred_element_type=f32)

    def t4(c, m):
        fm = pltpu.bitcast(DFT[pl.ds(0, 128), :], bf)
        w = _ld(UBv, c, pl.ds(64 * m, 64))
        UH[24 * c + m] = jnp.dot(fm, w, preferred_element_type=f32)

    def t5_row(base, r0, sign, link):
        re = pl.ds(r0, 8); im = pl.ds(128 + r0, 8)
        sr = si = None
        for j in range(16):
            if sr is None:
                i0r = i0i = None
                ar = link[0] - link[0]; ai = link[1] - link[1]
            else:
                i0r, i0i = -sign * si, sign * sr
                ar, ai = i0r, i0i
            for i in range(j + 1):
                kr = KH[base + i, re, :]; ki = KH[base + i, im, :]
                ur = UH[base + (j - i), re, :]; ui = UH[base + (j - i), im, :]
                ar = ar + kr * ur; ai = ai + kr * ui
                ar = ar - ki * ui; ai = ai + ki * ur
                yield
            trow = pl.ds(128 * (j % 2) + r0, 8)
            KH[base + (16 + j // 2), trow, :] = ar
            UH[base + (16 + j // 2), trow, :] = ai
            if i0r is None:
                sr, si = ar, ai
            else:
                sr, si = ar - i0r, ai - i0i
        link[0], link[1] = sr, si

    def t5_rows(base, rows, link):
        for (r0, sign) in rows:
            yield from t5_row(base, r0, sign, link)

    def t6(c, j):
        fi = jnp.concatenate([pltpu.bitcast(DFT[pl.ds(128, 64), :], bf),
                              pltpu.bitcast(DFT[pl.ds(192, 64), :], bf)], axis=1)
        tr = pl.ds(128 * (j % 2), 128) if isinstance(j, int) else pl.ds(pl.multiple_of(128 * (j % 2), 128), 128)
        w = jnp.concatenate([KH[24 * c + 16 + j // 2 + z0, tr, :],
                             UH[24 * c + 16 + j // 2 + z0, tr, :]], axis=0).astype(bf)
        y = jnp.dot(fi, w, preferred_element_type=f32)
        rows = pl.ds(128 * j, 128) if isinstance(j, int) else pl.ds(pl.multiple_of(128 * j, 128), 128)
        rows2 = pl.ds(64 * j, 64) if isinstance(j, int) else pl.ds(pl.multiple_of(64 * j, 64), 64)
        uu = _ld(UBv, c, rows2).astype(f32)
        OUT[4 + c, rows, :] = (y + uu * DSKB[c, pl.ds(0, 1), :]).astype(bf)

    def relayout(dst, srcv, t0_, t):
        for b in range(4):
            dst[t + z0, b] = _ld(srcv, t0_ + t, pl.ds(64 * b, 64)).T

    def xblk(j):
        return jnp.concatenate([_ld(XBv, b, pl.ds(64 * j, 64)) for b in range(4)], axis=1)

    def proj_k(j, g):
        k = jnp.dot(xblk(j), _ld(WBv, 4 + g), preferred_element_type=f32)
        kb = k.astype(bf)
        KS[g, pl.ds(128 * j, 128), :] = kb
        if j >= 2:
            kr = pltpu.roll(pltpu.bitcast(kb[64:128], i32), 16, 1)
            KR[g, pl.ds(64 * j, 64), :] = pltpu.bitcast(kr, bf)

    qscale = float(0.25 * np.log2(np.e))

    def proj_t(j, which):
        src = WQTv if which == 'q' else WVTv
        wt = jnp.concatenate([jnp.concatenate([_ld(src, g, b) for b in range(4)], axis=1) for g in range(4)],
                             axis=0)
        r = jax.lax.dot_general(wt, xblk(j), (((1,), (1,)), ((), ())), preferred_element_type=f32)
        if which == 'q':
            QT[j] = (r * qscale).astype(bf)
        else:
            VT[j] = r.astype(bf)

    zeros16 = jnp.zeros((16, 128), bf)

    def prod_unit(qi, h, kt, S, slot, macc):
        g, hh = h // 8, h % 8
        kb = qi - 2 + kt
        kk = _ld(KSv, g, _ds(64 * kb, 64))
        qh = _ld(QTv, qi, pl.ds(8 * h, 8))
        w = jnp.concatenate([zeros16] * hh + [qh] + [zeros16] * (7 - hh), axis=0)
        s = jnp.dot(kk, w, preferred_element_type=f32)
        if kt != 1:
            s = s + BIAS[kt // 2]
        S[slot] = s
        pm = jnp.max(s.reshape(16, 8, 128), axis=0)
        return pm if macc is None else jnp.maximum(macc, pm)

    def cons_unit(qi, h, kt, S, slot, m, lacc, oacc):
        kb = qi - 2 + kt
        p = jnp.exp2(S[slot] - m)
        ps = jnp.sum(p.reshape(16, 8, 128), axis=0)
        lacc = ps if lacc is None else lacc + ps
        v = _ld(VTv, kb, pl.ds(8 * h, 8))
        o = jnp.dot(v, p.astype(bf), preferred_element_type=f32)
        oacc = o if oacc is None else oacc + o
        return lacc, oacc

    def lane_iota(n):
        return jax.lax.broadcasted_iota(i32, (n, 128), 1)

    def tri_prod(qi, h, kt, S, slot, macc):
        g, hh = h // 8, h % 8
        qv = QTv[qi, pl.ds(8 * h, 8), :]
        z8 = jnp.zeros((8, 128), i32)
        if kt < 2:
            wv = jnp.concatenate([z8] * hh + [qv] + [z8] * (7 - hh), axis=0)
            if kt == 0:
                kv = jnp.concatenate([KSv[g, _ds(64 * qi, 32), :], KSv[g, _ds(64 * (qi - 2) + 32, 32), :]], axis=0)
            else:
                kv = KSv[g, _ds(64 * (qi - 1), 64), :]
        else:
            lo = lane_iota(8) < 64
            parts = [z8] * 8
            parts[hh] = jnp.where(lo, qv, 0)
            parts[(hh + 1) % 8] = jnp.where(lo, 0, qv)
            wv = jnp.concatenate(parts, axis=0)
            sel = (lane_iota(32) >> 4) == (hh + 1) % 8
            kv = jnp.where(sel, KRv[g, _ds(32 * qi, 32), :], KSv[g, _ds(64 * (qi - 2), 32), :])
        s = jnp.dot(pltpu.bitcast(kv, bf), pltpu.bitcast(wv, bf), preferred_element_type=f32)
        if kt == 0:
            s = s + BIAS[2]
        if kt == 2:
            s = s + BIAS[3, pl.ds(0, 64), :]
            S[slot, pl.ds(0, 64), :] = s
            pm = jnp.max(s.reshape(8, 8, 128), axis=0)
        else:
            S[slot] = s
            pm = jnp.max(s.reshape(16, 8, 128), axis=0)
        return pm if macc is None else jnp.maximum(macc, pm)

    def tri_cons(qi, h, kt, S, slot, m, lacc, oacc):
        if kt == 2:
            p = jnp.exp2(S[slot, pl.ds(0, 64), :] - m)
            ps = jnp.sum(p.reshape(8, 8, 128), axis=0)
            pv = pltpu.bitcast(p.astype(bf), i32)
            lo = lane_iota(32) < 64
            w = pltpu.bitcast(jnp.concatenate([jnp.where(lo, pv, 0), jnp.where(lo, 0, pv)], axis=0), bf)
        else:
            p = jnp.exp2(S[slot] - m)
            ps = jnp.sum(p.reshape(16, 8, 128), axis=0)
            w = p.astype(bf)
        lacc = ps if lacc is None else lacc + ps
        if kt == 1:
            v = VTv[qi - 1, pl.ds(8 * h, 8), :]
        else:
            va = VTv[qi - 2, pl.ds(8 * h, 8), :]
            vc = VTv[qi, pl.ds(8 * h, 8), :]
            lo8 = lane_iota(8) < 64
            v = jnp.where(lo8, vc, va) if kt == 0 else jnp.where(lo8, va, vc)
        o = jnp.dot(pltpu.bitcast(v, bf), w, preferred_element_type=f32)
        oacc = o if oacc is None else oacc + o
        return lacc, oacc

    def is_tri(qi):
        return (not isinstance(qi, int)) or qi >= 2

    def kts(qi):
        if is_tri(qi):
            return list(KT_ORDER)
        return [kt for kt in range(3) if qi - 2 + kt >= 0]

    def group(pitem, Sp, citem, Sc, ms, filler):
        new_ms = []
        for t in range(GS):
            macc = lacc = oacc = None
            pk_ = kts(pitem[0]) if pitem is not None else []
            ck_ = kts(citem[0]) if citem is not None else []
            for n in range(max(len(pk_), len(ck_))):
                for ph in (('c', 'p') if CONS_FIRST else ('p', 'c')):
                    if ph == 'p' and n < len(pk_):
                        pu = tri_prod if is_tri(pitem[0]) else prod_unit
                        macc = pu(pitem[0], GS * pitem[1] + t, pk_[n], Sp, 3 * t + pk_[n], macc)
                    if ph == 'c' and n < len(ck_):
                        cu = tri_cons if is_tri(citem[0]) else cons_unit
                        lacc, oacc = cu(citem[0], GS * citem[1] + t, ck_[n], Sc, 3 * t + ck_[n], ms[t], lacc, oacc)
                filler()
            if pitem is not None:
                new_ms.append(jnp.max(macc, axis=0, keepdims=True))
            if citem is not None:
                l = jnp.sum(lacc, axis=0, keepdims=True)
                o = oacc * pl.reciprocal(l, approx=True)
                h = GS * citem[1] + t
                OT[citem[0], pl.ds(16 * h, 16), :] = o.astype(bf)
        return new_ms

    def out_proj(i, g):
        wt = jnp.concatenate([_ld(WOTv, g, b) for b in range(4)], axis=1)
        r = jnp.dot(wt, _ld(OTv, i), preferred_element_type=f32)
        OUT[g, _ds(128 * i, 128), :] = r.astype(bf).T

    def out_cp(ct, r0, nr, si):
        return pltpu.make_async_copy(OUT.at[ct, _ds(r0, nr)],
                                     out_hbm.at[_ds(r0, nr), _ds(128 * ct, 128)], osems.at[si])

    mac = {}

    def fill():
        if RR:
            budget = {c: mac[c][1] for c in mac}
            while budget:
                for c in list(budget):
                    try:
                        next(mac[c][0])
                        budget[c] -= 1
                        if budget[c] <= 0:
                            del budget[c]
                    except StopIteration:
                        del mac[c]
                        del budget[c]
            return
        for c in list(mac):
            gen, rate = mac[c]
            for _ in range(rate):
                try:
                    next(gen)
                except StopIteration:
                    del mac[c]
                    break

    def drain(c):
        while c in mac:
            fill()

    cp_ldt.start()
    start(cp_par)
    start(cp_w[4:8])
    start(cp_x[0])
    start(cp_x[1])
    start(cp_w[0:4])
    start(cp_w[8:12])
    bias_init()

    links = [[jnp.zeros((8, 128), f32), jnp.zeros((8, 128), f32)] for _ in range(4)]
    next_row = [0, 0, 0, 0]

    def mac_rows(c, n, nfill):
        if n <= 0:
            return
        rows = [(8 * r, 1.0 if r < 8 else -1.0) for r in range(next_row[c], next_row[c] + n)]
        next_row[c] += n
        if SPLIT == 0:
            mac[c] = (t5_rows(24 * c + z0, rows, links[c]), int(np.ceil(136 * n / nfill)))
        else:
            for k in range(0, n, SPLIT):
                rr = rows[k:k + SPLIT]
                lk = [jnp.zeros((8, 128), f32), jnp.zeros((8, 128), f32)]
                mac[(c, k)] = (t5_rows(24 * c + z0, rr, lk), int(np.ceil(136 * len(rr) / nfill)))

    def drain_all():
        for c in list(mac):
            drain(c)

    def ssm_out(c, j0, j1):
        for j in range(j0, j1):
            t6(c, j)
            if j % 4 == 3:
                out_cp(4 + c, 128 * (j - 3), 512, 4 * c + j // 4).start()

    def block(p=None, vs=(), tabs=(), t2s=(), d34=(), macs=(), t6s=(), pre=None, nok=False):
        for (c, n) in macs:
            mac_rows(c, n, 6 if p is not None else 4)
        extra = []
        for c in t2s:
            extra += [(lambda c=c, ai=ai: t2(c, ai)) for ai in range(32)]
        for c in d34:
            for i in range(16):
                extra += [(lambda c=c, i=i: t3(c, i)), (lambda c=c, i=i: t4(c, i))]
        vands = []
        for g in vs:
            vands += [(lambda g=g, d=d: t1_vand(g, d, d + 8)) for d in range(0, 32, 8)]
        nv = (len(vands) + 3) // 4
        ne = (len(extra) + 3) // 4
        for g in range(4):
            if g < len(tabs):
                t1_tables(tabs[g])
            if p is not None:
                if not nok:
                    proj_k(p, g)
                fill()
            for f in vands[nv * g:nv * (g + 1)]:
                f()
            if p is not None and g == 1:
                proj_t(p, 'q')
                fill()
            if p is not None and g == 3:
                proj_t(p, 'v')
                fill()
            for f in extra[ne * g:ne * (g + 1)]:
                f()
            if p is None:
                fill()
            if pre is not None:
                pre(g)
        drain_all()
        for (c, j0, j1) in t6s:
            ssm_out(c, j0, j1)

    cp_ldt.wait(); wait(cp_par)
    for c in range(4):
        t0(c)
    t1_tables(0)
    wait(cp_w[4:8]); wait(cp_x[0])
    t1_tables(1)
    for g in range(4):
        proj_k(0, g)
    wait(cp_x[1])
    t1_tables(2)
    for j in (1, 2, 3):
        for g in range(4):
            proj_k(j, g)
    wait(cp_w[0:4])
    cp_dft.start(); start(cp_u); cp_mm.start(); start(cp_x[2]); start(cp_x[3]); start(cp_wo); cp_dsk.start()
    t1_tables(3)
    for t in range(4):
        relayout(WQT, WBv, 0, t)
    for d in range(0, 32, 8):
        t1_vand(0, d, d + 8)
    wait(cp_w[8:12])
    for t in range(4):
        relayout(WVT, WBv, 8, t)
    for d in range(0, 32, 8):
        t1_vand(1, d, d + 8)
    proj_t(0, 'q')
    proj_t(0, 'v')
    waits = {'x2': cp_x[2], 'x3': cp_x[3], 'u': [cp_dft, cp_mm] + cp_u, 'wo': cp_wo + [cp_dsk]}
    for blk in SCHED:
        blk = dict(blk)
        for w in blk.pop('wait', ()):
            wait(waits[w])
            if w == 'wo':
                dsk = DSK[...].astype(f32).reshape(1, D)
                for c in range(4):
                    DSKB[c] = jnp.broadcast_to(dsk[:, 128 * c:128 * (c + 1)], (8, 128))
        if blk.pop('wot', False):
            blk['pre'] = lambda g: relayout(WOT, WOBv, 0, g)
        block(**blk)
    assert next_row[0] == 16 and next_row[1] == 16 and next_row[2] == 16, next_row

    def qtile(qi, qnext, ms, hook, filler):
        bufs = [SA, SB]
        ng = 32 // GS
        for gi in range(ng):
            if gi < ng - 1:
                nxt = (qi, gi + 1)
            else:
                nxt = (qnext, 0) if qnext is not None else None
            ms = group(nxt, bufs[(gi + 1) % 2], (qi, gi), bufs[gi % 2], ms, filler)
            for hg in range(8 * gi // ng, 8 * (gi + 1) // ng):
                hook(hg)
        return ms

    ms = group((0, 0), SA, None, None, None, lambda: None)
    mac_rows(3, min(Q0_ROWS, 16 - next_row[3]), 32 + 12)
    ms = qtile(0, 1, ms, lambda hg: None, fill)
    drain_all()
    mac_rows(3, 16 - next_row[3], 64 + 20)

    def hook1(hg):
        if 1 <= hg < 5:
            out_proj(0, hg - 1)
        if not any(c == 2 for b in SCHED for (c, _, _) in b.get('t6s', ())):
            ssm_out(2, 2 * hg, 2 * hg + 2)
    ms = qtile(1, 2, ms, hook1, fill)
    drain_all()
    for g in range(4):
        out_cp(g, 0, 128, 16 + 16 * g).start()
    ssm_out(3, 0, 16)

    def body(it, ms):
        qi = it + 2

        def hook(hg):
            if 1 <= hg < 5:
                out_proj(qi - 1, hg - 1)
        ms = qtile(qi, jnp.minimum(qi + 1, 15), list(ms), hook, lambda: None)
        for g in range(4):
            out_cp(g, 128 * (qi - 1), 128, 16 + 16 * g + qi - 1).start()
        return tuple(ms)

    jax.lax.fori_loop(0, 14, body, tuple(ms), unroll=UNROLL)
    for g in range(4):
        out_proj(15, g)
        out_cp(g, 128 * 15, 128, 16 + 16 * g + 15).start()
    for c in range(4):
        for q4 in range(4):
            out_cp(4 + c, 512 * q4, 512, 4 * c + q4).wait()
    for g in range(4):
        for q in range(16):
            out_cp(g, 128 * q, 128, 16 + 16 * g + q).wait()


@jax.jit
def pallas_concat_heads__sliding_block__ssm_conv_s4__prompt_kernel(A_x, A_wqkv, A_wo, B_u, B_A_re, B_A_im, B_B_re, B_B_im, B_C_re, B_C_im, B_log_dt, B_Dskip):
    any_spec = pl.BlockSpec(memory_space=pl.ANY)
    scratch = [
        pltpu.VMEM((4, S_LEN, 128), bf), pltpu.VMEM((4, S_LEN, 128), bf), pltpu.VMEM((12, D, 128), bf),
        pltpu.VMEM((4, D, 128), bf),
        pltpu.VMEM((6, D, 128), bf), pltpu.VMEM((D,), bf), pltpu.VMEM((D,), bf),
        pltpu.VMEM((256, 128), i32), pltpu.VMEM((2048, 128), i32),
        pltpu.VMEM((4, 4, 128, 128), bf), pltpu.VMEM((4, 4, 128, 128), bf), pltpu.VMEM((4, 4, 128, 128), bf),
        pltpu.VMEM((NT, D, 128), bf), pltpu.VMEM((4, S_LEN, 128), bf), pltpu.VMEM((4, S_LEN // 2, 128), bf),
        pltpu.VMEM((NT, D, 128), bf),
        pltpu.VMEM((NT, D, 128), bf), pltpu.VMEM((3 * GS, 128, 128), f32), pltpu.VMEM((3 * GS, 128, 128), f32),
        pltpu.VMEM((4, 128, 128), f32),
        pltpu.VMEM((NTB, 2, 40 * SR, 128), i32), pltpu.VMEM((D * SR + 4 * D, 128), f32),
        pltpu.VMEM((4, 32, 48, 128), f32), pltpu.VMEM((96, 256, 128), f32), pltpu.VMEM((96, 256, 128), f32),
        pltpu.VMEM((4, 8, 128), f32), pltpu.VMEM((8, S_LEN, 128), bf),
        pltpu.SemaphoreType.DMA((48,)), pltpu.SemaphoreType.DMA((80,)),
    ]
    out = pl.pallas_call(
        _kernel,
        out_shape=jax.ShapeDtypeStruct((S_LEN, 2 * D), bf),
        in_specs=[pl.BlockSpec(memory_space=pltpu.SMEM)] + [any_spec] * 14,
        out_specs=any_spec,
        scratch_shapes=scratch,
        compiler_params=pltpu.CompilerParams(vmem_limit_bytes=110 * 1024 * 1024, flags=FLAGS or None),
        name="fused_swa_s4",
    )(_ZERO, A_x.reshape(S_LEN, D), A_wqkv, A_wo, B_u.reshape(S_LEN, D), B_A_re, B_A_im, B_B_re, B_B_im, B_C_re, B_C_im,
      B_log_dt, B_Dskip, _DFT_CONST, _M_CONST)
    return out.reshape(1, S_LEN, 2 * D)
```

```python
import numpy as np
import jax
import jax.numpy as jnp
import jax.experimental.pallas as pl
import jax.experimental.pallas.tpu as pltpu

S_LEN = 2048
D = 512
NT = 16
NEG = -1e30
bf = jnp.bfloat16
f32 = jnp.float32
i32 = jnp.int32

A_EXP = list(range(16)) + list(range(16, 32, 2)) + list(range(32, 64, 4))
B_EXP = ([16 * b for b in range(16)] + [258 + 32 * b for b in range(8)]
         + [516 + 64 * b for b in range(8)] + [1032 + 64 * b for b in range(16)])
WIN_OF_BLOCK = [0, 1, 2, 3, 4, 5, 5, 5, 6, 7, 7, 7, 7, 7, 7, 7]


def _bf16_bits(x):
    x = np.ascontiguousarray(np.asarray(x, np.float32))
    u = x.view(np.uint32).astype(np.uint64)
    return ((u + 0x7FFF + ((u >> 16) & 1)) >> 16).astype(np.uint32)


def _pack_rows(x):
    b = _bf16_bits(x)
    return (b[0::2] | (b[1::2] << 16)).astype(np.uint32).view(np.int32)


def _windows():
    ai_of = {e: i for i, e in enumerate(A_EXP)}
    W0 = [(ai, 0) for ai in range(16)]
    W1 = [(ai, 8) for ai in range(16)]
    W2 = [(ai_of[e], 16) for e in range(0, 32, 2)]
    W3 = [(ai_of[e], 24) for e in range(0, 64, 4)]
    W4 = [(ai_of[e], 32) for e in range(0, 64, 8)] + [(ai_of[e], 40) for e in range(0, 64, 8)]

    def cols(W):
        return [A_EXP[ai] + B_EXP[b0 + r] for (ai, b0) in W for r in range(8)]
    c2s = cols(W2); c2s[7] = A_EXP[16] + B_EXP[15]
    c3s = cols(W3); c3s[7] = A_EXP[23] + B_EXP[23]
    c4s = cols(W4); c4s[7] = A_EXP[31] + B_EXP[31]
    return [cols(W0), cols(W1), c2s, cols(W2), c3s, cols(W3), c4s, cols(W4)]


def _make_consts():
    k = np.concatenate([np.arange(0, 128, 2), np.arange(1, 128, 2)]).astype(np.float64) + 0.5
    t = np.arange(128, dtype=np.float64)
    th = 2 * np.pi * k[:, None] * t[None, :] / 256
    F = np.concatenate([np.cos(th), -np.sin(th)], axis=0)
    Finv = np.concatenate([np.cos(th).T, -np.sin(th).T], axis=1) / 128
    wins = _windows()
    M = np.zeros((16, 256, 128))
    for i in range(16):
        lag = (_bf16_bits(np.arange(128 * i, 128 * i + 128)) << 16).view(np.float32).astype(np.int64)
        w = wins[WIN_OF_BLOCK[i]]
        for tt in range(128):
            M[i, :, w.index(int(lag[tt]))] += F[:, tt]
    dft = np.concatenate([_pack_rows(F), _pack_rows(Finv[:, :128]), _pack_rows(Finv[:, 128:])], axis=0)
    mm = np.concatenate([_pack_rows(M[i]) for i in range(16)], axis=0)
    return np.ascontiguousarray(dft), np.ascontiguousarray(mm)


_DFT_CONST, _M_CONST = _make_consts()
_ZERO = np.zeros((8,), np.int32)


def _cmul(a, b):
    return (a[0] * b[0] - a[1] * b[1], a[0] * b[1] + a[1] * b[0])


def _cmul_conj(a, b):
    return (a[0] * b[0] + a[1] * b[1], a[1] * b[0] - a[0] * b[1])


def _csq(a):
    return (a[0] * a[0] - a[1] * a[1], 2.0 * (a[0] * a[1]))


def _pk(x, y):
    return pltpu.pack_elementwise([x, y], packed_dtype=bf)


def _sincos(x):
    kf = (x * 0.6366197723675814 + 12582912.0) - 12582912.0
    r = ((x - kf * 1.5703125) - kf * 4.837512969970703125e-4) - kf * 7.54978995489188216e-8
    ki = kf.astype(i32)
    z = r * r
    s = r + (r * z) * (-1.6666654611e-1 + z * (8.3321608736e-3 + z * -1.9515295891e-4))
    c = (1.0 - 0.5 * z) + (z * z) * (4.166664568298827e-2 + z * (-1.388731625493765e-3 + z * 2.443315711809948e-5))
    swap = (ki & 1) != 0
    sn = jnp.where(swap, c, s)
    cs = jnp.where(swap, s, c)
    sbit = jnp.int32(-2 ** 31)
    sn = pltpu.bitcast(pltpu.bitcast(sn, i32) ^ ((ki << 30) & sbit), f32)
    cs = pltpu.bitcast(pltpu.bitcast(cs, i32) ^ (((ki + 1) << 30) & sbit), f32)
    return sn, cs


SR = 33
GCH = 32
NTB = 6
TB = 16
ZOFF = D * SR
UNROLL = 7


def _ds(start, n):
    return pl.ds(start if isinstance(start, int) else pl.multiple_of(start, n), n)


def _v(ref):
    return ref.bitcast(i32)


def _ld(view, *idx):
    return pltpu.bitcast(view[idx], bf)


SCHED = [
    dict(vs=(2, 3), tabs=(4, 5, 6)),
    dict(vs=(4, 5, 6), tabs=(7, 8, 9)),
    dict(vs=(7, 8, 9), tabs=(10, 11, 12)),
    dict(wait=('u',), vs=(10, 11, 12), tabs=(13, 14, 15), t2s=(0,), d34=(0,)),
    dict(vs=(13, 14, 15), d34=(1,), macs=((0, 3),)),
    dict(p=1, nok=True, t2s=(2,), d34=(2,), macs=((0, 3), (1, 3))),
    dict(p=2, nok=True, d34=(3,), macs=((0, 3), (1, 3))),
    dict(p=3, nok=True, macs=((0, 2), (1, 2))),
    dict(wait=('x2', 'wo'), p=4, macs=((0, 2), (1, 2), (2, 1))),
    dict(p=5, macs=((0, 2), (1, 2), (2, 1))),
    dict(p=6, macs=((0, 1), (1, 2), (2, 2))),
    dict(p=7, macs=((1, 2), (2, 2)), t6s=((0, 0, 8),)),
    dict(wait=('x3',), p=8, macs=((2, 2), (3, 2)), t6s=((0, 8, 16),)),
    dict(p=9, macs=((2, 2), (3, 2)), t6s=((1, 0, 8),)),
    dict(p=10, macs=((2, 2), (3, 2)), t6s=((1, 8, 16),)),
    dict(p=11, macs=((2, 2), (3, 2))),
    dict(p=12, macs=((2, 2), (3, 2))),
    dict(p=13, macs=((3, 2),), t6s=((2, 0, 8),)),
    dict(p=14, macs=((3, 2),), t6s=((2, 8, 16),)),
    dict(p=15, macs=((3, 2),), wot=True),
]
GS = 4


def _kernel(zero_ref, x_hbm, wqkv_hbm, wo_hbm, u_hbm, are_hbm, aim_hbm, bre_hbm, bim_hbm, cre_hbm, cim_hbm,
            ldt_hbm, dsk_hbm, dft_hbm, mm_hbm,
            out_hbm,
            XB, UB, WB, WOB, PAR, LDT, DSK, DFT, MM,
            WQT, WVT, WOT,
            QT, KS, KR, VT, OT, SA, SB, BIAS,
            TAB, XG, XT, KH, UH, DSKB, OUT,
            sems, osems):
    z0 = zero_ref[0]
    XBv, UBv, WBv, WOBv = _v(XB), _v(UB), _v(WB), _v(WOB)
    WQTv, WVTv, WOTv = _v(WQT), _v(WVT), _v(WOT)
    QTv, KSv, KRv, VTv, OTv = _v(QT), _v(KS), _v(KR), _v(VT), _v(OT)
    nsem = [0]

    def mk(src, dst):
        cp = pltpu.make_async_copy(src, dst, sems.at[nsem[0]])
        nsem[0] += 1
        return cp
    par_src = [are_hbm, aim_hbm, bre_hbm, bim_hbm, cre_hbm, cim_hbm]
    cp_par = [mk(par_src[i].at[pl.ds(0, 256)], PAR.at[i, pl.ds(0, 256)]) for i in range(6)]
    cp_par2 = [mk(par_src[i].at[pl.ds(256, 256)], PAR.at[i, pl.ds(256, 256)]) for i in range(6)]
    cp_ldt = mk(ldt_hbm, LDT)
    cp_dsk = mk(dsk_hbm, DSK)
    cp_w = [mk(wqkv_hbm.at[:, pl.ds(128 * t, 128)], WB.at[t]) for t in range(12)]
    x_chunks = [(0, 128), (128, 384), (512, 512), (1024, 1024)]
    cp_x = [[mk(x_hbm.at[pl.ds(r0, nr), pl.ds(128 * b, 128)], XB.at[b, pl.ds(r0, nr)])
             for b in range(4)] for (r0, nr) in x_chunks]
    cp_u = [mk(u_hbm.at[:, pl.ds(128 * b, 128)], UB.at[b]) for b in range(4)]
    cp_wo = [mk(wo_hbm.at[:, pl.ds(128 * b, 128)], WOB.at[b]) for b in range(4)]
    cp_dft = mk(dft_hbm, DFT)
    cp_mm = mk(mm_hbm, MM)

    def start(l):
        for c in l:
            c.start()

    def wait(l):
        for c in l:
            c.wait()

    def bias_init():
        kk = jax.lax.broadcasted_iota(i32, (128, 128), 0)
        qq = jax.lax.broadcasted_iota(i32, (128, 128), 1)
        BIAS[0] = jnp.where(kk > qq, 0.0, NEG).astype(f32)
        BIAS[1] = jnp.where(kk <= qq, 0.0, NEG).astype(f32)
        BIAS[2] = jnp.where(kk < 64, jnp.where(kk <= qq, 0.0, NEG), jnp.where(kk > qq, 0.0, NEG)).astype(f32)
        BIAS[3] = jnp.where(qq < 64, jnp.where(kk > qq, 0.0, NEG), jnp.where(kk + 64 <= qq, 0.0, NEG)).astype(f32)

    def t0(c):
        dtr = LDT[...].astype(f32).reshape(1, D)
        dtr = jnp.exp(dtr[:, 128 * c:128 * (c + 1)]).astype(bf).astype(f32)
        dtc = jnp.broadcast_to(dtr, (128, 128)).T
        for b in range(8):
            rows = pl.ds(128 * c + 16 * b, 16)
            dt = dtc[16 * b:16 * (b + 1)]
            are = PAR[0, rows, :].astype(f32); aim = PAR[1, rows, :].astype(f32)
            bre = PAR[2, rows, :].astype(f32) * dt; bim = PAR[3, rows, :].astype(f32) * dt
            cre = PAR[4, rows, :].astype(f32); cim = PAR[5, rows, :].astype(f32)
            mag = jnp.exp(dt * are)
            sn, cs = _sincos(dt * aim)
            r0 = ZOFF + 128 * c + 16 * b
            XG[pl.ds(r0, 16), :] = mag * cs
            XG[pl.ds(r0 + D, 16), :] = mag * sn
            XG[pl.ds(r0 + 2 * D, 16), :] = cre * bre - cim * bim
            XG[pl.ds(r0 + 3 * D, 16), :] = -(cre * bim + cim * bre)

    def t1_tables(g):
        buf = g % NTB
        for blk in range(GCH // TB):
            r0 = ZOFF + 256 * (g // 8) + 128 * blk + 16 * (g % 8)

            def zc(k, r0=r0):
                return XG[pl.ds(pl.multiple_of(8 * z0 + (r0 + k * D), 8), TB), :]
            z = (zc(0), zc(1))
            cur = (zc(2), zc(3))
            pend = []

            def emit(base, idx, v, blk=blk, pend=pend):
                if idx % 2 == 0:
                    pend.append(v)
                else:
                    v0 = pend.pop()
                    q = base + idx // 2
                    TAB[buf, 0, pl.ds(q * SR + TB * blk, TB), :] = _pk(v0[0], v[0])
                    TAB[buf, 1, pl.ds(q * SR + TB * blk, TB), :] = _pk(v0[1], v[1])
            z2 = _csq(z); z4 = _csq(z2)
            n = 0
            emit(0, n, cur); n += 1
            for (mult, cnt) in ((z, 16), (z2, 8), (z4, 7)):
                for _ in range(cnt):
                    cur = _cmul_conj(cur, mult)
                    emit(0, n, cur); n += 1
            z8 = _csq(z4); z16 = _csq(z8); z32 = _csq(z16)
            n = 0
            emit(16, n, (jnp.ones_like(z[0]), jnp.zeros_like(z[0]))); n += 1
            emit(16, n, z16); n += 1
            emit(16, n, z32); n += 1
            cur = z32
            for b in range(3, 16):
                cur = _cmul(cur, z16)
                if b == 4:
                    z64 = cur
                emit(16, n, cur); n += 1
            cur = _cmul(_cmul(cur, z16), z2)
            z258 = cur
            emit(16, n, cur); n += 1
            for _ in range(7):
                cur = _cmul(cur, z32)
                emit(16, n, cur); n += 1
            cur = _csq(z258); z516 = cur
            emit(16, n, cur); n += 1
            for _ in range(7):
                cur = _cmul(cur, z64)
                emit(16, n, cur); n += 1
            cur = _csq(z516)
            emit(16, n, cur); n += 1
            for _ in range(15):
                cur = _cmul(cur, z64)
                emit(16, n, cur); n += 1

    def t1_vand(g, d0, d1):
        buf = g % NTB

        def ld(ri, base, n, d):
            return jnp.concatenate(
                [pltpu.bitcast(TAB[buf, ri, pl.ds((base + 8 * j) * SR + d, 8, stride=SR), :], bf)
                 for j in range(n)], axis=0)

        def ab(d):
            return (jnp.concatenate([ld(0, 0, 2, d), ld(1, 0, 2, d)], axis=1),
                    jnp.concatenate([ld(0, 16, 3, d), ld(1, 16, 3, d)], axis=1))
        nt = (((1,), (1,)), ((), ()))
        z16 = jnp.zeros((16, 256), bf)
        lo = jax.lax.broadcasted_iota(i32, (32, 128), 1) < 64
        for d in range(d0 // 2, d1 // 2):
            a0, b0 = ab(d)
            a1, b1 = ab(16 + d)
            o = jax.lax.dot_general(jnp.concatenate([a0, a1], axis=0),
                                    jnp.concatenate([b0, z16, b1, z16], axis=0), nt,
                                    preferred_element_type=f32)
            XG[pl.ds((128 * (g // 8) + 16 * (g % 8) + d) * SR, 32), :] = jnp.where(lo, o[0:32], o[32:64])

    def t2(c, ai):
        tt = XG[pl.ds(128 * (c // 2) * SR + ai, 128, stride=SR), :].T
        XT[c, ai] = tt[0:48]
        XT[c + 1, ai] = tt[64:112]

    ai_of = {e: i for i, e in enumerate(A_EXP)}
    wgroups = [[(ai, 0) for ai in range(16)], [(ai, 8) for ai in range(16)],
               [(ai_of[e], 16) for e in range(0, 32, 2)], [(ai_of[e], 24) for e in range(0, 64, 4)],
               [(ai_of[e], 32) for e in range(0, 64, 8)] + [(ai_of[e], 40) for e in range(0, 64, 8)]]
    wins = [(wgroups[0], None), (wgroups[1], None), (wgroups[2], (16, 8)), (wgroups[2], None),
            (wgroups[3], (23, 16)), (wgroups[3], None), (wgroups[4], (31, 24)), (wgroups[4], None)]

    def t3(c, i):
        grp, edge = wins[WIN_OF_BLOCK[i]]
        parts = [XT[c, ai, pl.ds(b0, 8), :] for (ai, b0) in grp]
        if edge is not None:
            sub7 = jax.lax.broadcasted_iota(i32, (8, 128), 0) == 7
            parts[0] = jnp.where(sub7, XT[c, edge[0], pl.ds(edge[1], 8), :], parts[0])
        w = jnp.concatenate(parts, axis=0).astype(bf)
        m = pltpu.bitcast(MM[pl.ds(128 * i, 128), :], bf)
        KH[24 * c + i] = jnp.dot(m, w, preferred_element_type=f32)

    def t4(c, m):
        fm = pltpu.bitcast(DFT[pl.ds(0, 128), :], bf)
        w = _ld(UBv, c, pl.ds(64 * m, 64))
        UH[24 * c + m] = jnp.dot(fm, w, preferred_element_type=f32)

    def t5_row(base, r0, sign, link):
        re = pl.ds(r0, 8); im = pl.ds(128 + r0, 8)
        sr = si = None
        for j in range(16):
            if sr is None:
                i0r = i0i = None
                ar = link[0] - link[0]; ai = link[1] - link[1]
            else:
                i0r, i0i = -sign * si, sign * sr
                ar, ai = i0r, i0i
            for i in range(j + 1):
                kr = KH[base + i, re, :]; ki = KH[base + i, im, :]
                ur = UH[base + (j - i), re, :]; ui = UH[base + (j - i), im, :]
                ar = ar + kr * ur; ai = ai + kr * ui
                ar = ar - ki * ui; ai = ai + ki * ur
                yield
            trow = pl.ds(128 * (j % 2) + r0, 8)
            KH[base + (16 + j // 2), trow, :] = ar
            UH[base + (16 + j // 2), trow, :] = ai
            if i0r is None:
                sr, si = ar, ai
            else:
                sr, si = ar - i0r, ai - i0i
        link[0], link[1] = sr, si

    def t5_rows(base, rows, link):
        for (r0, sign) in rows:
            yield from t5_row(base, r0, sign, link)

    def t6(c, j):
        fi = jnp.concatenate([pltpu.bitcast(DFT[pl.ds(128, 64), :], bf),
                              pltpu.bitcast(DFT[pl.ds(192, 64), :], bf)], axis=1)
        tr = pl.ds(128 * (j % 2), 128) if isinstance(j, int) else pl.ds(pl.multiple_of(128 * (j % 2), 128), 128)
        w = jnp.concatenate([KH[24 * c + 16 + j // 2 + z0, tr, :],
                             UH[24 * c + 16 + j // 2 + z0, tr, :]], axis=0).astype(bf)
        y = jnp.dot(fi, w, preferred_element_type=f32)
        rows = pl.ds(128 * j, 128) if isinstance(j, int) else pl.ds(pl.multiple_of(128 * j, 128), 128)
        rows2 = pl.ds(64 * j, 64) if isinstance(j, int) else pl.ds(pl.multiple_of(64 * j, 64), 64)
        uu = _ld(UBv, c, rows2).astype(f32)
        OUT[4 + c, rows, :] = (y + uu * DSKB[c, pl.ds(0, 1), :]).astype(bf)

    def relayout(dst, srcv, t0_, t):
        for b in range(4):
            dst[t + z0, b] = _ld(srcv, t0_ + t, pl.ds(64 * b, 64)).T

    def xblk(j):
        return jnp.concatenate([_ld(XBv, b, pl.ds(64 * j, 64)) for b in range(4)], axis=1)

    def proj_k(j, g):
        k = jnp.dot(xblk(j), _ld(WBv, 4 + g), preferred_element_type=f32)
        kb = k.astype(bf)
        KS[g, pl.ds(128 * j, 128), :] = kb
        if j >= 2:
            kr = pltpu.roll(pltpu.bitcast(kb[64:128], i32), 16, 1)
            KR[g, pl.ds(64 * j, 64), :] = pltpu.bitcast(kr, bf)

    qscale = float(0.25 * np.log2(np.e))

    def proj_t(j, which):
        src = WQTv if which == 'q' else WVTv
        wt = jnp.concatenate([jnp.concatenate([_ld(src, g, b) for b in range(4)], axis=1) for g in range(4)],
                             axis=0)
        r = jax.lax.dot_general(wt, xblk(j), (((1,), (1,)), ((), ())), preferred_element_type=f32)
        if which == 'q':
            QT[j] = (r * qscale).astype(bf)
        else:
            VT[j] = r.astype(bf)

    zeros16 = jnp.zeros((16, 128), bf)

    def prod_unit(qi, h, kt, S, slot, macc):
        g, hh = h // 8, h % 8
        kb = qi - 2 + kt
        kk = _ld(KSv, g, _ds(64 * kb, 64))
        qh = _ld(QTv, qi, pl.ds(8 * h, 8))
        w = jnp.concatenate([zeros16] * hh + [qh] + [zeros16] * (7 - hh), axis=0)
        s = jnp.dot(kk, w, preferred_element_type=f32)
        if kt != 1:
            s = s + BIAS[kt // 2]
        S[slot] = s
        pm = jnp.max(s.reshape(16, 8, 128), axis=0)
        return pm if macc is None else jnp.maximum(macc, pm)

    def cons_unit(qi, h, kt, S, slot, m, lacc, oacc):
        kb = qi - 2 + kt
        p = jnp.exp2(S[slot] - m)
        ps = jnp.sum(p.reshape(16, 8, 128), axis=0)
        lacc = ps if lacc is None else lacc + ps
        v = _ld(VTv, kb, pl.ds(8 * h, 8))
        o = jnp.dot(v, p.astype(bf), preferred_element_type=f32)
        oacc = o if oacc is None else oacc + o
        return lacc, oacc

    def lane_iota(n):
        return jax.lax.broadcasted_iota(i32, (n, 128), 1)

    def tri_prod(qi, h, kt, S, slot, macc):
        g, hh = h // 8, h % 8
        qv = QTv[qi, pl.ds(8 * h, 8), :]
        z8 = jnp.zeros((8, 128), i32)
        if kt < 2:
            wv = jnp.concatenate([z8] * hh + [qv] + [z8] * (7 - hh), axis=0)
            if kt == 0:
                kv = jnp.concatenate([KSv[g, _ds(64 * qi, 32), :], KSv[g, _ds(64 * (qi - 2) + 32, 32), :]], axis=0)
            else:
                kv = KSv[g, _ds(64 * (qi - 1), 64), :]
        else:
            lo = lane_iota(8) < 64
            parts = [z8] * 8
            parts[hh] = jnp.where(lo, qv, 0)
            parts[(hh + 1) % 8] = jnp.where(lo, 0, qv)
            wv = jnp.concatenate(parts, axis=0)
            sel = (lane_iota(32) >> 4) == (hh + 1) % 8
            kv = jnp.where(sel, KRv[g, _ds(32 * qi, 32), :], KSv[g, _ds(64 * (qi - 2), 32), :])
        s = jnp.dot(pltpu.bitcast(kv, bf), pltpu.bitcast(wv, bf), preferred_element_type=f32)
        if kt == 0:
            s = s + BIAS[2]
        if kt == 2:
            s = s + BIAS[3, pl.ds(0, 64), :]
            S[slot, pl.ds(0, 64), :] = s
            pm = jnp.max(s.reshape(8, 8, 128), axis=0)
        else:
            S[slot] = s
            pm = jnp.max(s.reshape(16, 8, 128), axis=0)
        return pm if macc is None else jnp.maximum(macc, pm)

    def tri_cons(qi, h, kt, S, slot, m, lacc, oacc):
        if kt == 2:
            p = jnp.exp2(S[slot, pl.ds(0, 64), :] - m)
            ps = jnp.sum(p.reshape(8, 8, 128), axis=0)
            pv = pltpu.bitcast(p.astype(bf), i32)
            lo = lane_iota(32) < 64
            w = pltpu.bitcast(jnp.concatenate([jnp.where(lo, pv, 0), jnp.where(lo, 0, pv)], axis=0), bf)
        else:
            p = jnp.exp2(S[slot] - m)
            ps = jnp.sum(p.reshape(16, 8, 128), axis=0)
            w = p.astype(bf)
        lacc = ps if lacc is None else lacc + ps
        if kt == 1:
            v = VTv[qi - 1, pl.ds(8 * h, 8), :]
        else:
            va = VTv[qi - 2, pl.ds(8 * h, 8), :]
            vc = VTv[qi, pl.ds(8 * h, 8), :]
            lo8 = lane_iota(8) < 64
            v = jnp.where(lo8, vc, va) if kt == 0 else jnp.where(lo8, va, vc)
        o = jnp.dot(pltpu.bitcast(v, bf), w, preferred_element_type=f32)
        oacc = o if oacc is None else oacc + o
        return lacc, oacc

    def is_tri(qi):
        return (not isinstance(qi, int)) or qi >= 2

    def kts(qi):
        if is_tri(qi):
            return [0, 1, 2]
        return [kt for kt in range(3) if qi - 2 + kt >= 0]

    def group(pitem, Sp, citem, Sc, ms, filler):
        new_ms = []
        for t in range(GS):
            macc = lacc = oacc = None
            pk_ = kts(pitem[0]) if pitem is not None else []
            ck_ = kts(citem[0]) if citem is not None else []
            for n in range(max(len(pk_), len(ck_))):
                for ph in ('p', 'c'):
                    if ph == 'p' and n < len(pk_):
                        pu = tri_prod if is_tri(pitem[0]) else prod_unit
                        macc = pu(pitem[0], GS * pitem[1] + t, pk_[n], Sp, 3 * t + pk_[n], macc)
                    if ph == 'c' and n < len(ck_):
                        cu = tri_cons if is_tri(citem[0]) else cons_unit
                        lacc, oacc = cu(citem[0], GS * citem[1] + t, ck_[n], Sc, 3 * t + ck_[n], ms[t], lacc, oacc)
                filler()
            if pitem is not None:
                new_ms.append(jnp.max(macc, axis=0, keepdims=True))
            if citem is not None:
                l = jnp.sum(lacc, axis=0, keepdims=True)
                o = oacc * pl.reciprocal(l, approx=True)
                h = GS * citem[1] + t
                OT[citem[0], pl.ds(16 * h, 16), :] = o.astype(bf)
        return new_ms

    def out_proj(i, g):
        wt = jnp.concatenate([_ld(WOTv, g, b) for b in range(4)], axis=1)
        r = jnp.dot(wt, _ld(OTv, i), preferred_element_type=f32)
        OUT[g, _ds(128 * i, 128), :] = r.astype(bf).T

    def out_cp(ct, r0, nr, si):
        return pltpu.make_async_copy(OUT.at[ct, _ds(r0, nr)],
                                     out_hbm.at[_ds(r0, nr), _ds(128 * ct, 128)], osems.at[si])

    mac = {}

    def fill():
        for c in list(mac):
            gen, rate = mac[c]
            for _ in range(rate):
                try:
                    next(gen)
                except StopIteration:
                    del mac[c]
                    break

    def drain(c):
        while c in mac:
            fill()

    cp_ldt.start()
    start(cp_par)
    start(cp_w[4:8])
    start(cp_x[0])
    start(cp_x[1])
    start(cp_w[0:4])
    start(cp_w[8:12])
    start(cp_par2)
    bias_init()

    links = [[jnp.zeros((8, 128), f32), jnp.zeros((8, 128), f32)] for _ in range(4)]
    next_row = [0, 0, 0, 0]

    def mac_rows(c, n, nfill):
        if n <= 0:
            return
        rows = [(8 * r, 1.0 if r < 8 else -1.0) for r in range(next_row[c], next_row[c] + n)]
        next_row[c] += n
        mac[c] = (t5_rows(24 * c + z0, rows, links[c]), int(np.ceil(136 * n / nfill)))

    def drain_all():
        for c in list(mac):
            drain(c)

    def ssm_out(c, j0, j1):
        for j in range(j0, j1):
            t6(c, j)
            if j % 4 == 3:
                out_cp(4 + c, 128 * (j - 3), 512, 4 * c + j // 4).start()

    def block(p=None, vs=(), tabs=(), t2s=(), d34=(), macs=(), t6s=(), pre=None, nok=False):
        for (c, n) in macs:
            mac_rows(c, n, 6 if p is not None else 4)
        extra = []
        for c in t2s:
            extra += [(lambda c=c, ai=ai: t2(c, ai)) for ai in range(32)]
        for c in d34:
            for i in range(16):
                extra += [(lambda c=c, i=i: t3(c, i)), (lambda c=c, i=i: t4(c, i))]
        vands = []
        for g in vs:
            vands += [(lambda g=g, d=d: t1_vand(g, d, d + 8)) for d in range(0, 32, 8)]
        nv = (len(vands) + 3) // 4
        ne = (len(extra) + 3) // 4
        for g in range(4):
            if g < len(tabs):
                t1_tables(tabs[g])
            if p is not None:
                if not nok:
                    proj_k(p, g)
                fill()
            for f in vands[nv * g:nv * (g + 1)]:
                f()
            if p is not None and g == 1:
                proj_t(p, 'q')
                fill()
            if p is not None and g == 3:
                proj_t(p, 'v')
                fill()
            for f in extra[ne * g:ne * (g + 1)]:
                f()
            if p is None:
                fill()
            if pre is not None:
                pre(g)
        drain_all()
        for (c, j0, j1) in t6s:
            ssm_out(c, j0, j1)

    cp_ldt.wait(); wait(cp_par)
    t0(0)
    t0(1)
    t1_tables(0)
    wait(cp_w[4:8]); wait(cp_x[0])
    t1_tables(1)
    for g in range(4):
        proj_k(0, g)
    wait(cp_x[1])
    t1_tables(2)
    for j in (1, 2, 3):
        for g in range(4):
            proj_k(j, g)
    wait(cp_w[0:4])
    cp_dft.start(); start(cp_u); cp_mm.start(); start(cp_x[2]); start(cp_x[3]); start(cp_wo); cp_dsk.start()
    t1_tables(3)
    for t in range(4):
        relayout(WQT, WBv, 0, t)
    for d in range(0, 32, 8):
        t1_vand(0, d, d + 8)
    wait(cp_w[8:12])
    for t in range(4):
        relayout(WVT, WBv, 8, t)
    for d in range(0, 32, 8):
        t1_vand(1, d, d + 8)
    proj_t(0, 'q')
    wait(cp_par2)
    t0(2)
    t0(3)
    proj_t(0, 'v')
    waits = {'x2': cp_x[2], 'x3': cp_x[3], 'u': [cp_dft, cp_mm] + cp_u, 'wo': cp_wo + [cp_dsk]}
    for blk in SCHED:
        blk = dict(blk)
        for w in blk.pop('wait', ()):
            wait(waits[w])
            if w == 'wo':
                dsk = DSK[...].astype(f32).reshape(1, D)
                for c in range(4):
                    DSKB[c] = jnp.broadcast_to(dsk[:, 128 * c:128 * (c + 1)], (8, 128))
        if blk.pop('wot', False):
            blk['pre'] = lambda g: relayout(WOT, WOBv, 0, g)
        block(**blk)
    assert next_row[0] == 16 and next_row[1] == 16 and next_row[2] == 16, next_row

    def qtile(qi, qnext, ms, hook, filler):
        bufs = [SA, SB]
        ng = 32 // GS
        for gi in range(ng):
            if gi < ng - 1:
                nxt = (qi, gi + 1)
            else:
                nxt = (qnext, 0) if qnext is not None else None
            ms = group(nxt, bufs[(gi + 1) % 2], (qi, gi), bufs[gi % 2], ms, filler)
            for hg in range(8 * gi // ng, 8 * (gi + 1) // ng):
                hook(hg)
        return ms

    ms = group((0, 0), SA, None, None, None, lambda: None)
    mac_rows(3, 16 - next_row[3], 32 + 12)
    ms = qtile(0, 1, ms, lambda hg: None, fill)
    drain_all()
    mac_rows(3, 16 - next_row[3], 64 + 20)

    def hook1(hg):
        if 1 <= hg < 5:
            out_proj(0, hg - 1)
    ms = qtile(1, 2, ms, hook1, fill)
    drain_all()
    for g in range(4):
        out_cp(g, 0, 128, 16 + 16 * g).start()
    ssm_out(3, 0, 16)

    def body(it, ms):
        qi = it + 2

        def hook(hg):
            if 1 <= hg < 5:
                out_proj(qi - 1, hg - 1)
        ms = qtile(qi, jnp.minimum(qi + 1, 15), list(ms), hook, lambda: None)
        for g in range(4):
            out_cp(g, 128 * (qi - 1), 128, 16 + 16 * g + qi - 1).start()
        return tuple(ms)

    jax.lax.fori_loop(0, 14, body, tuple(ms), unroll=UNROLL)
    for g in range(4):
        out_proj(15, g)
        out_cp(g, 128 * 15, 128, 16 + 16 * g + 15).start()
    for c in range(4):
        for q4 in range(4):
            out_cp(4 + c, 512 * q4, 512, 4 * c + q4).wait()
    for g in range(4):
        for q in range(16):
            out_cp(g, 128 * q, 128, 16 + 16 * g + q).wait()


@jax.jit
def pallas_concat_heads__sliding_block__ssm_conv_s4__prompt_kernel(A_x, A_wqkv, A_wo, B_u, B_A_re, B_A_im, B_B_re, B_B_im, B_C_re, B_C_im, B_log_dt, B_Dskip):
    any_spec = pl.BlockSpec(memory_space=pl.ANY)
    scratch = [
        pltpu.VMEM((4, S_LEN, 128), bf), pltpu.VMEM((4, S_LEN, 128), bf), pltpu.VMEM((12, D, 128), bf),
        pltpu.VMEM((4, D, 128), bf),
        pltpu.VMEM((6, D, 128), bf), pltpu.VMEM((D,), bf), pltpu.VMEM((D,), bf),
        pltpu.VMEM((256, 128), i32), pltpu.VMEM((2048, 128), i32),
        pltpu.VMEM((4, 4, 128, 128), bf), pltpu.VMEM((4, 4, 128, 128), bf), pltpu.VMEM((4, 4, 128, 128), bf),
        pltpu.VMEM((NT, D, 128), bf), pltpu.VMEM((4, S_LEN, 128), bf), pltpu.VMEM((4, S_LEN // 2, 128), bf),
        pltpu.VMEM((NT, D, 128), bf),
        pltpu.VMEM((NT, D, 128), bf), pltpu.VMEM((3 * GS, 128, 128), f32), pltpu.VMEM((3 * GS, 128, 128), f32),
        pltpu.VMEM((4, 128, 128), f32),
        pltpu.VMEM((NTB, 2, 40 * SR, 128), i32), pltpu.VMEM((D * SR + 4 * D, 128), f32),
        pltpu.VMEM((4, 32, 48, 128), f32), pltpu.VMEM((96, 256, 128), f32), pltpu.VMEM((96, 256, 128), f32),
        pltpu.VMEM((4, 8, 128), f32), pltpu.VMEM((8, S_LEN, 128), bf),
        pltpu.SemaphoreType.DMA((56,)), pltpu.SemaphoreType.DMA((80,)),
    ]
    out = pl.pallas_call(
        _kernel,
        out_shape=jax.ShapeDtypeStruct((S_LEN, 2 * D), bf),
        in_specs=[pl.BlockSpec(memory_space=pltpu.SMEM)] + [any_spec] * 14,
        out_specs=any_spec,
        scratch_shapes=scratch,
        compiler_params=pltpu.CompilerParams(vmem_limit_bytes=110 * 1024 * 1024),
        name="fused_swa_s4",
    )(_ZERO, A_x.reshape(S_LEN, D), A_wqkv, A_wo, B_u.reshape(S_LEN, D), B_A_re, B_A_im, B_B_re, B_B_im, B_C_re, B_C_im,
      B_log_dt, B_Dskip, _DFT_CONST, _M_CONST)
    return out.reshape(1, S_LEN, 2 * D)
```
